```python
import os as _os
_os.environ.setdefault("JAX_PLATFORMS", "cpu")
import jax
import jax.numpy as jnp

def _softmax(x, axis=-1):
    return jax.nn.softmax(x, axis=axis)
def _gelu(x):
    return jax.nn.gelu(x, approximate=True)
def _silu(x):
    return jax.nn.silu(x)
def _sigmoid(x):
    return jax.nn.sigmoid(x)
def _layernorm(x, axis=-1, eps=1e-5):
    m = jnp.mean(x, axis=axis, keepdims=True)
    v = jnp.var(x, axis=axis, keepdims=True)
    return (x - m) / jnp.sqrt(v + eps)
def _scatter_add(tgt, idx, src, axis=0):
    return tgt.at[idx].add(src)
def _segment_sum(src, seg, n):
    return jax.ops.segment_sum(src, seg, n)
class _Rng:
    def __init__(self, key):
        self._k = key
    def _next(self):
        self._k, sub = jax.random.split(self._k)
        return sub
    def normal(self, shape):
        return jax.random.normal(self._next(), shape, dtype=jnp.bfloat16)
    def randint(self, lo, hi, shape):
        return jax.random.randint(self._next(), shape, lo, hi, dtype=jnp.int32)
    def uniform(self, shape, lo=0.0, hi=1.0):
        return jax.random.uniform(self._next(), shape, jnp.bfloat16, lo, hi)
    def permutation(self, n):
        return jax.random.permutation(self._next(), n)


kernel_name = 'interleave_layers__ssm_conv_h3__linear_attn_block__prompt'

def setup_inputs():
    _rng = _Rng(jax.random.key(int.from_bytes(__import__("os").urandom(4), "little")))
    _w = (lambda a: (lambda t: t.astype(jnp.bfloat16) if jnp.issubdtype(t.dtype, jnp.floating) else t)(jnp.asarray(a)))
    def _A_setup():
        B, S, D = 1, 2048, 512
        ks = 4
        return {
            "q": _w((lambda *s: _rng.normal(s) * 0.05)(B, S, D)),
            "k": _w((lambda *s: _rng.normal(s) * 0.4)(B, S, D)),
            "v": _w((lambda *s: _rng.normal(s) * 0.4)(B, S, D)),
            "shift_k": _w((lambda *s: _rng.normal(s) * 0.4)(D, ks) * 0.5),
            "ssm_k": _w((lambda *s: _rng.normal(s) * 0.4)(D, S) * (1.0 / S ** 0.5)),
            "ssm_D": _w((lambda *s: _rng.normal(s) * 0.4)(D)),
        }
    _A_in = _A_setup()

    def _B_setup():
        B, S, D = 1, 2048, 512
        return {
            "x": _w((lambda *s: _rng.normal(s) * 0.05)(B, S, D)),
            "wqkv": _w((lambda *s: _rng.normal(s) * 0.1)(D, 3 * D)),
            "wo": _w((lambda *s: _rng.normal(s) * 0.1)(D, D)),
        }
    _B_in = _B_setup()

    return {
        "A_q": _A_in["q"],
        "A_k": _A_in["k"],
        "A_v": _A_in["v"],
        "A_shift_k": _A_in["shift_k"],
        "A_ssm_k": _A_in["ssm_k"],
        "A_ssm_D": _A_in["ssm_D"],
        "B_x": _B_in["x"],
        "B_wqkv": _B_in["wqkv"],
        "B_wo": _B_in["wo"],
    }

def reference(A_q, A_k, A_v, A_shift_k, A_ssm_k, A_ssm_D, B_x, B_wqkv, B_wo):
    def _A_ref(q, k, v, shift_k, ssm_k, ssm_D):
        B, S, D = q.shape
        ks = shift_k.shape[-1]
        k_pad = jnp.pad(k, ((0, 0), (ks - 1, 0), (0, 0)))
        k_shift = jnp.zeros_like(k)
        for t in range(ks):
            k_shift = k_shift + k_pad[:, t:t + S, :] * shift_k[:, ks - 1 - t][None, None, :]
        kv = k_shift * v
        L = 2 * S
        kv_pad = jnp.pad(kv, ((0, 0), (0, S), (0, 0)))
        kf_pad = jnp.pad(ssm_k, ((0, 0), (0, S)))
        kv_f = (lambda x, axes=(-2,-1): jnp.fft.rfft2(x.astype(jnp.float32), axes=axes))(kv_pad[:, None, :, :], axes=(1, 2))
        kf_f = (lambda x, axes=(-2,-1): jnp.fft.rfft2(x.astype(jnp.float32), axes=axes))(kf_pad[:, None, :], axes=(1, 2))
        kf_f = (lambda x, *d: x.transpose(*d))(kf_f, 1, 2, 0)
        y_f = kv_f * kf_f[None, :, :, :]
        y = (lambda x, s, axes=(-2,-1): jnp.fft.irfft2(x, s=s, axes=axes).astype(jnp.bfloat16))(y_f, (1, L), axes=(1, 2))[:, 0, :S, :]
        y = y + kv * ssm_D[None, None, :]
        return q * y

    def _B_ref(x, wqkv, wo):
        B, S, D = x.shape
        H = 32; Dh = D // H
        qkv = (lambda x, *d: x.transpose(*d))((x @ wqkv).reshape(B, S, 3, H, Dh), 2, 0, 3, 1, 4)
        q, k, v = qkv[0], qkv[1], qkv[2]
        phi = lambda t: jnp.where(t > 0, t + 1, jnp.exp(t)) + 1e-6
        pq, pk = phi(q), phi(k)
        kv = jnp.einsum("bhsd,bhse->bhde", pk, v)
        z = jnp.einsum("bhsd->bhd", pk)
        num = jnp.einsum("bhqd,bhde->bhqe", pq, kv)
        den = jnp.einsum("bhqd,bhd->bhq", pq, z)[..., None] + 1e-6
        o = num / den
        return (lambda x, *d: x.transpose(*d))(o, 0, 2, 1, 3).reshape(B, S, D) @ wo

    x = A_q
    x = x + _A_ref(_layernorm(x, axis=-1), A_k, A_v, A_shift_k, A_ssm_k, A_ssm_D)
    x = x + _B_ref(_layernorm(x, axis=-1), B_wqkv, B_wo)
    x = x + _A_ref(_layernorm(x, axis=-1), A_k, A_v, A_shift_k, A_ssm_k, A_ssm_D)
    x = x + _B_ref(_layernorm(x, axis=-1), B_wqkv, B_wo)
    return x
```

```python
import functools
import os
import numpy as np
import jax
import jax.numpy as jnp
from jax import lax
import jax.experimental.pallas as pl
import jax.experimental.pallas.tpu as pltpu

S, D = 2048, 512
P = 128
NB = S // P
NF = 2 * P
HF = P // 2
NH, DH = 32, 16
RB = 256
NR = S // RB
LT = D // 128
HW = D // 2
F32 = jnp.float32
BF16 = jnp.bfloat16
U32 = jnp.uint32
STOP = int(os.environ.get('STOP', '9'))
KVG = 32


def _consts():
    n = np.arange(P)
    rows = []
    for par in range(2):
        f = np.arange(par, P, 2)
        ph = ((2 * f[:, None] + 1) * n[None, :]) % (4 * P)
        th = 2.0 * np.pi * ph / (4 * P)
        rows += [np.cos(th), -np.sin(th)]
    ff = np.concatenate(rows, axis=0)
    fi = ff.T * (2.0 / NF)
    korder = [par * P + ri * HF + f for par in range(2) for f in range(HF) for ri in range(2)]
    fi = fi[:, korder]
    torder = [g * KVG + h * (KVG // 2) + r for g in range(P // KVG) for r in range(KVG // 2) for h in range(2)]
    ffu = ff[:, torder]
    pm = np.zeros((128, 128), np.float32)
    for hl in range(8):
        for e in range(16):
            pm[e * 8 + hl, hl * 16 + e] = 1.0
    return np.concatenate([ff, fi[:, :P], fi[:, P:], pm, ffu], axis=0).astype(np.float32)


def _ln(x):
    m = jnp.mean(x, axis=-1, keepdims=True)
    xc = x - m
    v = jnp.mean(xc * xc, axis=-1, keepdims=True)
    return xc * lax.rsqrt(v + 1e-5)


def _phi(t):
    return jnp.where(t > 0, t + 1.0, jnp.exp(t)) + 1e-6


def _dot(a, b):
    return jnp.dot(a, b, preferred_element_type=F32)


def _dot_nt(a, b):
    return lax.dot_general(a, b, (((1,), (1,)), ((), ())), preferred_element_type=F32)


def _pk(x):
    return pltpu.bitcast(x, U32)


def _upk(x):
    return pltpu.bitcast(x, BF16)


def _pack2(a, b):
    return pltpu.bitcast(pltpu.pack_elementwise([a, b], packed_dtype=BF16), F32)


CST = HF + 8
SLOT = 3 * CST
AREA = 2 * SLOT
SP_ROWS = 2 * LT * AREA
PSLOT = 4 * CST
PAREA = NR * PSLOT
WPK = 2 * LT * PAREA
PW_ROWS = WPK + 2 * 2 * LT * P
YTOK = LT * S
YA_ROWS = YTOK + 8
ASK = LT * (S // 2)
KVB_ROWS = ASK + 4 * LT * 8
NTICK = 1024


def _sp(c, par):
    return (c * 2 + par) * AREA


def _pw(c, par, p):
    return (c * 2 + par) * PAREA + p * PSLOT


def _wrow(p, o, c):
    return WPK + (((p % 2) * 2 + o) * LT + c) * P


def _kernel(q_hbm, k_hbm, v_hbm, sk_hbm, h_hbm, sd_hbm, w_hbm, wo_hbm, c_hbm, z_hbm,
            o_hbm,
            q_v, k_v, v_v, h_v, w_v, wo_v, o_v, sk_v, sd_v, c_v, z_sm,
            cu_s, kf_s, hraw_s, tk_s, pw, ya, kvb, xn_s, x_s, pq_s, g_s, z_s,
            wqk_s, m_s, zr_s,
            sem_in, sem_o, *spb):
    su, sh = spb[:NR], spb[NR:]

    def cp_rows(src, dst, i):
        return lambda s: pltpu.make_async_copy(src.at[0, pl.ds(i * RB, RB), :], dst.at[pl.ds(i * RB, RB), :], s)

    ck = lambda i: cp_rows(k_hbm, k_v, i)
    cv = lambda i: cp_rows(v_hbm, v_v, i)
    cq = lambda i: cp_rows(q_hbm, q_v, i)
    ch = lambda i, n=1: (lambda s: pltpu.make_async_copy(h_hbm.at[:, pl.ds(i * RB, n * RB)], h_v.at[:, pl.ds(i * RB, n * RB)], s))
    cw = lambda i: (lambda s: pltpu.make_async_copy(w_hbm.at[:, pl.ds(i * D, D)], w_v.at[:, pl.ds(i * D, D)], s))
    full = lambda a, b: (lambda s: pltpu.make_async_copy(a, b, s))
    groups = [
        [full(z_hbm, z_sm)],
        [full(c_hbm, c_v), full(sk_hbm, sk_v), full(sd_hbm, sd_v), ch(0), ck(0), cv(0)],
        [ch(1), ck(1), cv(1), cq(0), cw(1)],
        [ch(2, 3), ck(2), cv(2), cq(1), ck(3), cv(3)],
        [ch(5, 3), ck(4), cv(4), cq(2), cw(0)],
        [ck(5), cv(5), cq(3)],
        [ck(6), cv(6), cq(4)],
        [ck(7), cv(7), cq(5)],
        [cq(6)],
        [cq(7), cw(2), full(wo_hbm, wo_v)],
    ]
    for gi, g in enumerate(groups):
        for c in g:
            c(sem_in.at[gi]).start()

    ticks = []

    def wait(gi):
        for c in groups[gi]:
            c(sem_in.at[gi]).wait()
        del ticks[:]

    def cp_o(i): return pltpu.make_async_copy(o_v.at[pl.ds(i * RB, RB), :], o_hbm.at[0, pl.ds(i * RB, RB), :], sem_o.at[0])

    for c in range(LT):
        kf_s[c, 0:8, :] = jnp.zeros((8, 128), F32)
    g_s[...] = jnp.zeros_like(g_s)
    z_s[...] = jnp.zeros_like(z_s)

    wait(0); wait(1)
    zero = z_sm[0]
    never = jnp.full((8, 128), zero, jnp.int32) != 0
    cu_s[...] = _pk(c_v[...])
    ff = lambda: _upk(cu_s[0:128, :])
    fi = lambda: jnp.concatenate([_upk(cu_s[128:192, :]), _upk(cu_s[192:256, :])], axis=1)
    pm = lambda: _upk(cu_s[256:320, :])
    ffu = lambda: _upk(cu_s[320:448, :])

    def ldd(buf, r, n=8):
        return buf[pl.ds(pl.multiple_of(r + zero, 8), n), :]

    for b in spb:
        b[pl.ds(pl.multiple_of(HF + zero, 8), 8), :] = jnp.zeros((8, 128), F32)

    def tick(val, order):
        for (r, c) in order:
            ticks.append(val[r * 8:(r + 1) * 8, c * 128:(c + 1) * 128])

    def tk_at(frac):
        return ticks[min(int(frac * len(ticks)), len(ticks) - 1)]

    skf = sk_v[...].astype(F32)
    for t in range(4):
        for c in range(LT):
            r = ASK + (t * LT + c) * 8
            kvb[r:r + 8, :] = jnp.broadcast_to(skf[t:t + 1, c * 128:(c + 1) * 128], (8, 128))

    def put3(buf, hf, par, slot, comps):
        for m, val in enumerate(comps):
            for cl in range(2):
                r = _sp(2 * hf + cl, par) + slot * SLOT + m * CST
                buf[r:r + HF, :] = val[:, cl * 128:(cl + 1) * 128]

    def t_kv(i, n=32, t0=None, t1=None):
        r0 = i * RB
        items = [(hf, b0) for hf in range(2) for b0 in range(r0, r0 + RB, n)]
        for k, (hf, b0) in enumerate(items):
            kf2 = k_v[b0:b0 + n, hf * HW:(hf + 1) * HW].astype(F32)
            vf2 = v_v[b0:b0 + n, hf * HW:(hf + 1) * HW].astype(F32)
            for cl in range(2):
                c = 2 * hf + cl
                sk = [kvb[ASK + (t * LT + c) * 8:ASK + (t * LT + c) * 8 + 8, :] for t in range(4)]
                if t0 is not None:
                    tk = tk_at(t0 + (t1 - t0) * (2 * k + cl) / (2 * len(items)))
                    sk = [jnp.where(never, tk, x) for x in sk]
                sk = [jnp.tile(x, (n // 8, 1)) for x in sk]
                kf = kf2[:, cl * 128:(cl + 1) * 128]
                kf_s[c, 8 + b0:8 + b0 + n, :] = kf
                ks = (kf * sk[0] + kf_s[c, 7 + b0:7 + b0 + n, :] * sk[1]
                      + kf_s[c, 6 + b0:6 + b0 + n, :] * sk[2] + kf_s[c, 5 + b0:5 + b0 + n, :] * sk[3])
                kv = ks * vf2[:, cl * 128:(cl + 1) * 128]
                for g in range(n // KVG):
                    r = c * (S // 2) + (b0 + g * KVG) // 2
                    kvb[r:r + KVG // 2, :] = _pack2(kv[g * KVG:g * KVG + KVG // 2], kv[g * KVG + KVG // 2:(g + 1) * KVG])

    def t_u(i):
        for hf in range(2):
            for hb in range(2):
                b0 = i * RB + hb * P
                kv = jnp.concatenate([_upk(ldd(kvb, c * (S // 2) + b0 // 2, P // 2)) for c in (2 * hf, 2 * hf + 1)], axis=1)
                u = _dot(ffu(), kv)
                tick(u, [(r, 0) for r in range(0, 32, 4)])
                for par in range(2):
                    ur, ui = u[par * P:par * P + HF], u[par * P + HF:(par + 1) * P]
                    put3(su[i], hf, par, hb, (ur, ui, ur + ui))

    def t_h(i):
        for hf in range(2):
            prev = hraw_s[:, hf * HW:(hf + 1) * HW] if i > 0 else None
            for j in (2 * i, 2 * i + 1):
                hh = _dot_nt(ff(), h_v[hf * HW:(hf + 1) * HW, j * P:(j + 1) * P])
                tick(hh, [(r, 0) for r in range(0, 32, 4)])
                if j == 0:
                    sd = sd_v[...].astype(F32).reshape(1, D)[:, hf * HW:(hf + 1) * HW]
                    hh = jnp.concatenate([hh[0:HF] + sd, hh[HF:P], hh[P:P + HF] + sd, hh[P + HF:NF]], axis=0)
                for par in range(2):
                    hr, hi = hh[par * P:par * P + HF], hh[par * P + HF:(par + 1) * P]
                    if prev is not None:
                        qr, qi = prev[par * P:par * P + HF], prev[par * P + HF:(par + 1) * P]
                        hr, hi = (hr - qi, hi + qr) if par == 0 else (hr + qi, hi - qr)
                    put3(sh[i], hf, par, j % 2, (hr, hi - hr, hi + hr))
                prev = hh
            if i < NR - 1:
                hraw_s[:, hf * HW:(hf + 1) * HW] = prev

    def mac_slab(p, a_lo, a_hi, first, c, par, f0, link):
        base = _sp(c, par) + f0
        pb = _pw(c, par, p) + f0
        lds = lambda buf, r: buf[pl.ds(pl.multiple_of(r, 8), 8), :]
        ldu = lambda a, m: lds(su[a // 2], base + (a % 2) * SLOT + m * CST)
        ldh = lambda j, m: lds(sh[j // 2], base + (j % 2) * SLOT + m * CST)
        pbs = lambda m: pl.ds(pl.multiple_of(pb + m * CST, 8), 8)

        def chain(hm, um, acc0, acc1, sign):
            h_prev = None
            for a in range(a_lo, a_hi + 1):
                u = ldu(a, um)
                h1 = h_prev if h_prev is not None else ldh(2 * p + 1 - a, hm)
                acc1 = acc1 + h1 * u if sign > 0 else acc1 - h1 * u
                if a <= 2 * p:
                    h0 = ldh(2 * p - a, hm)
                    acc0 = acc0 + h0 * u if sign > 0 else acc0 - h0 * u
                    h_prev = h0
            return acc0, acc1

        zz = jnp.zeros((8, 128), F32)
        b0, b1 = (zz, zz) if first else (pw[pbs(1), :], pw[pbs(3), :])
        b0, b1 = jnp.where(never, link, b0), jnp.where(never, link, b1)
        a0, a1 = chain(1, 0, b0, b1, 1)
        i0, i1 = chain(0, 2, a0, a1, 1)
        if first:
            k0, k1 = i0 - a0, i1 - a1
        else:
            k0, k1 = i0 + (pw[pbs(0), :] - a0), i1 + (pw[pbs(2), :] - a1)
        r0, r1 = chain(2, 1, k0, k1, -1)
        if a_hi == 2 * p + 1:
            pw[pl.ds(pl.multiple_of(_wrow(p, 0, c) + par * HF + f0, 8), 8), :] = _pack2(r0, i0)
            pw[pl.ds(pl.multiple_of(_wrow(p, 1, c) + par * HF + f0, 8), 8), :] = _pack2(r1, i1)
        else:
            for m, val in enumerate((r0, i0, r1, i1)):
                pw[pbs(m), :] = val
        return a1

    started = set()
    ntk = [0]

    def mac(p, a_lo, a_hi, t0=None, t1=None):
        first = p not in started
        started.add(p)
        base = ntk[0]
        if t0 is not None:
            ntk[0] += 64
            for k in range(64):
                tk_s[(base + k) * 8:(base + k + 1) * 8, :] = tk_at(t0 + (t1 - t0) * k / 64)
        link = jnp.zeros((8, 128), F32)
        for c in range(LT):
            for par in range(2):
                def body(ft, carry):
                    if t0 is not None:
                        carry = tk_s[pl.ds(pl.multiple_of((base + (c * 2 + par) * 8 + ft) * 8, 8), 8), :]
                    return mac_slab(p, a_lo, a_hi, first, c, par, ft * 8, carry)
                link = lax.fori_loop(0, HF // 8, body, link, unroll=True)

    def new(p, t0=None, t1=None):
        mac(p, max(2 * p - 4, 0), 2 * p + 1, t0, t1)

    def t_inv(i):
        for o in range(2):
            w = jnp.concatenate([_upk(ldd(pw, _wrow(i, o, c), P)) for c in range(LT)], axis=1)
            r0 = i * RB + o * P
            y = _dot(fi(), w)
            tick(y, [(r, c) for c in (1, 3) for r in range(0, 16, 2)])
            for c in range(LT):
                ya[c * S + r0:c * S + r0 + P, :] = y[:, c * 128:(c + 1) * 128]

    def ln_rows(r0, n, x, chained):
        if chained:
            y = jnp.concatenate([ldd(ya, c * S + r0, n) for c in range(LT)], axis=1)
        else:
            y = jnp.concatenate([ya[c * S + r0:c * S + r0 + n, :] for c in range(LT)], axis=1)
        x = x + _ln(x) * y
        x_s[r0:r0 + n, :] = x
        xnf = _ln(x)
        xn_s[r0 // 2:(r0 + n) // 2, :] = _pk(xnf.astype(BF16))
        if chained:
            tok = xnf[0:8, 0:128]
            for g in range(1, n // 8):
                tok = tok + xnf[g * 8:(g + 1) * 8, (g % LT) * 128:(g % LT + 1) * 128]
            ya[YTOK:YTOK + 8, :] = tok

    def t_ln(i, sizes=(32,) * 8):
        r0 = i * RB
        for n in sizes:
            ln_rows(r0, n, q_v[r0:r0 + n, :].astype(F32), True)
            r0 += n

    def ln_chain(i, x):
        ln_rows(i * RB, RB, x, False)

    def xn(i):
        return _upk(xn_s[i * RB // 2:(i + 1) * RB // 2, :])

    def t_q(i, n0=0, n1=D):
        r0 = i * RB
        qq = _dot_nt(xn(i), _upk(wqk_s[n0 // 2:n1 // 2, :]))
        tick(qq, [(r, c) for c in range((n1 - n0) // 128) for r in range(0, 32, 2)])
        pq_s[r0:r0 + RB, n0:n1] = _phi(qq).astype(BF16)

    def qp(i, n0=0, n1=LT):
        for n in range(n0, n1):
            t_q(i, n * 128, (n + 1) * 128)

    def t_kg(i):
        kt = _dot_nt(_upk(wqk_s[D // 2:D, :]), xn(i))
        pkt = _phi(kt)
        z_s[...] += pkt[:, :128] + pkt[:, 128:]
        g_s[...] += _dot(pkt.astype(BF16), xn(i))

    def kgp(i):
        st = {}

        def kt(m):
            kt = _dot_nt(_upk(wqk_s[D // 2 + m * 64:D // 2 + (m + 1) * 64, :]), xn(i))
            tick(kt, [(r, c) for c in range(2) for r in range(0, 16, 2)])
            pkt = _phi(kt)
            z_s[m * 128:(m + 1) * 128, :] += pkt[:, :128] + pkt[:, 128:]
            st[m] = pkt.astype(BF16)

        def gm(m):
            gg = _dot(st[m], xn(i))
            tick(gg, [(r, c) for c in (1, 3) for r in range(0, 16, 2)])
            g_s[m * 128:(m + 1) * 128, :] += gg
        kt(0)
        for m in range(4):
            if m + 1 < 4:
                kt(m + 1)
            gm(m)

    def wprep(part):
        blk = [_dot_nt(pm(), w_v[:, part * D + g * 128: part * D + (g + 1) * 128]) for g in range(4)]
        for g in range(4):
            tick(blk[g], [(r, 0) for r in range(0, 16, 2)])
        for e in range(16):
            rows = jnp.concatenate([blk[g][e * 8:(e + 1) * 8] for g in range(4)], axis=0)
            wqk_s[part * (D // 2) + e * 16: part * (D // 2) + (e + 1) * 16, :] = _pk(rows.astype(BF16))

    def finalize(last):
        zt = z_s[...].T
        zr_s[...] = jnp.broadcast_to(jnp.sum(zt, axis=0, keepdims=True), (8, D))
        rr = lax.broadcasted_iota(jnp.int32, (128, 128), 0) % 8
        cc = lax.broadcasted_iota(jnp.int32, (128, 128), 1) // DH
        mask = rr == cc
        ms = []
        for g in range(4):
            gg = jnp.concatenate([g_s[e * 32 + g * 8: e * 32 + g * 8 + 8, :] for e in range(16)], axis=0).astype(BF16)
            wv = w_v[:, 2 * D + g * 128: 2 * D + (g + 1) * 128]
            kvg = jnp.where(mask, _dot(gg, wv), 0.0).astype(BF16)
            ms.append(_dot(kvg, wo_v[g * 128:(g + 1) * 128, :]))
        for e in range(16):
            rows = jnp.concatenate([ms[g][e * 8:(e + 1) * 8] for g in range(4)], axis=0)
            m_s[e * 16:(e + 1) * 16, :] = _pk(rows.astype(BF16))
        if not last:
            g_s[...] = jnp.zeros_like(g_s)
            z_s[...] = jnp.zeros_like(z_s)

    def s5_att(i):
        r0 = i * RB
        pq = pq_s[r0:r0 + RB, :].astype(F32)
        t = pq * zr_s[0:1, :]
        t = (t[:, 0:128] + t[:, 128:256]) + (t[:, 256:384] + t[:, 384:512])
        t = t + pltpu.roll(t, 64, 1)
        t = t + pltpu.roll(t, 32, 1)
        den = t + 1e-6
        r = pl.reciprocal(den, approx=True)
        r = r * (2.0 - den * r)
        a = (pq * jnp.concatenate([r] * LT, axis=1)).astype(BF16)
        return x_s[r0:r0 + RB, :] + _dot(a, _upk(m_s[...]))

    t_h(0); t_kv(0, 128); t_u(0); new(0)
    wait(2)
    t_inv(0); t_h(1); t_kv(1, 128); t_u(1); t_ln(0, (128, 128)); new(1); wprep(1)
    wait(3)
    t_inv(1); t_h(2); t_kv(2, 128); t_u(2); kgp(0); t_h(3); t_h(4)
    t_ln(1); t_kv(3, 32, 0.6, 0.97); new(2, 0.35, 0.96)
    wait(4)
    t_inv(2); t_u(3); kgp(1); t_h(5); t_h(6); t_h(7); wprep(0)
    t_ln(2); t_kv(4, 32, 0.6, 0.97); mac(3, 0, 1, 0.0, 0.18); mac(4, 0, 3, 0.18, 0.5); new(3, 0.5, 0.96)
    wait(5)
    t_inv(3); t_u(4); qp(0); qp(1, 0, 2); kgp(2)
    t_ln(3); t_kv(5, 32, 0.6, 0.97); mac(5, 0, 5, 0.0, 0.48); new(4, 0.48, 0.96)
    wait(6)
    t_inv(4); t_u(5); qp(1, 2, 4); qp(2); kgp(3)
    t_ln(4); t_kv(6, 32, 0.6, 0.97); mac(6, 0, 5, 0.0, 0.48); new(5, 0.48, 0.96)
    wait(7)
    t_inv(5); t_u(6); qp(3); qp(4, 0, 2); kgp(4)
    t_ln(5); t_kv(7, 32, 0.6, 0.97); mac(6, 6, 7, 0.0, 0.18); mac(7, 0, 3, 0.18, 0.5); new(6, 0.5, 0.96)
    wait(8)
    t_inv(6); t_u(7); qp(4, 2, 4); qp(5); kgp(5)
    t_ln(6); mac(7, 4, 9, 0.0, 0.48); new(7, 0.48, 0.96)
    wait(9)
    t_inv(7); t_ln(7, (128, 128)); t_kg(6); t_q(6); t_kg(7); t_q(7)
    if STOP == 1:
        o_v[0:RB, :] = (g_s[0:RB, :] + x_s[S - RB:S, :] + z_s[0:RB, 0:1]).astype(BF16) + pq_s[S - RB:S, :]
        cp_o(0).start(); cp_o(0).wait()
        return
    finalize(False)

    ln_chain(0, s5_att(0))
    for i in range(NR):
        if i + 1 < NR:
            x = s5_att(i + 1)
        t_kg(i)
        if i + 1 < NR:
            ln_chain(i + 1, x)
        t_q(i)
    finalize(True)

    for i in range(NR):
        o_v[i * RB:(i + 1) * RB, :] = s5_att(i).astype(BF16)
        cp_o(i).start()
    for i in range(NR):
        cp_o(i).wait()


@jax.jit
def pallas_interleave_layers__ssm_conv_h3__linear_attn_block__prompt_kernel(
        A_q, A_k, A_v, A_shift_k, A_ssm_k, A_ssm_D, B_x, B_wqkv, B_wo):
    c = jnp.asarray(_consts(), BF16)
    z = jnp.asarray(np.zeros((8,), np.int32))
    any_spec = pl.BlockSpec(memory_space=pl.ANY)
    return pl.pallas_call(
        _kernel,
        out_shape=jax.ShapeDtypeStruct((1, S, D), BF16),
        in_specs=[any_spec] * 10,
        out_specs=any_spec,
        scratch_shapes=[
            pltpu.VMEM((S, D), BF16),
            pltpu.VMEM((S, D), BF16),
            pltpu.VMEM((S, D), BF16),
            pltpu.VMEM((D, S), BF16),
            pltpu.VMEM((D, 3 * D), BF16),
            pltpu.VMEM((D, D), BF16),
            pltpu.VMEM((S, D), BF16),
            pltpu.VMEM((4, D), BF16),
            pltpu.VMEM((D,), BF16),
            pltpu.VMEM((896, P), BF16),
            pltpu.SMEM((8,), jnp.int32),
            pltpu.VMEM((448, P), U32),
            pltpu.VMEM((LT, 8 + S, 128), F32),
            pltpu.VMEM((NF, D), F32),
            pltpu.VMEM((NTICK * 8, 128), F32),
            pltpu.VMEM((PW_ROWS, 128), F32),
            pltpu.VMEM((YA_ROWS, 128), F32),
            pltpu.VMEM((KVB_ROWS, 128), F32),
            pltpu.VMEM((S // 2, D), U32),
            pltpu.VMEM((S, D), F32),
            pltpu.VMEM((S, D), BF16),
            pltpu.VMEM((D, D), F32),
            pltpu.VMEM((D, 128), F32),
            pltpu.VMEM((D, D), U32),
            pltpu.VMEM((D // 2, D), U32),
            pltpu.VMEM((8, D), F32),
            pltpu.SemaphoreType.DMA((10,)),
            pltpu.SemaphoreType.DMA((1,)),
        ] + [pltpu.VMEM((SP_ROWS, 128), F32)] * (2 * NR),
        compiler_params=pltpu.CompilerParams(vmem_limit_bytes=110 * 1024 * 1024),
    )(A_q, A_k, A_v, A_shift_k.T, A_ssm_k, A_ssm_D, B_wqkv, B_wo, c, z)
```

```python
import functools
import numpy as np
import jax
import jax.numpy as jnp
from jax import lax
import jax.experimental.pallas as pl
import jax.experimental.pallas.tpu as pltpu

S, D = 2048, 512
RB = 256
NR = S // RB
NFQ = 256
HB = RB // 2
DH = 16
LT = D // 128
HW = D // 2
F32 = jnp.float32
BF16 = jnp.bfloat16
U32 = jnp.uint32
TAIL = 14
LN_OPS = 1900.0


C_FH, C_OH, C_FU, C_CE, C_SO, C_PM, C_ROWS = 0, 512, 528, 1040, 1296, 1552, 1680


def _iota(shape, d):
    return lax.broadcasted_iota(jnp.int32, shape, d)


def _cossin(row_a, row_step, col, scale=None):
    nt, w = row_a.shape[0], col.shape[1]
    ang = lambda ph: (ph & 2047).astype(F32) * np.float32(np.pi / 1024.0)
    ta = ang(row_a * col)
    tb = ang(_iota((8, w), 0) * row_step * col)
    ca, sa, cb, sb = jnp.cos(ta), jnp.sin(ta), jnp.cos(tb), jnp.sin(tb)
    if scale is not None:
        cb, sb = cb * scale, sb * scale
    cs = [ca[t:t + 1] * cb - sa[t:t + 1] * sb for t in range(nt)]
    sn = [sa[t:t + 1] * cb + ca[t:t + 1] * sb for t in range(nt)]
    return jnp.concatenate(cs, axis=0), jnp.concatenate(sn, axis=0)


def _gen_consts(put):
    t = _iota((32, 1), 0)
    fa = 64 * (t % 8) + 2 * (t // 8) + 1
    p = _iota((1, 128), 1)
    c, sn = _cossin(fa, 8, jnp.where(p == 0, 2 * HB, 2 * p), jnp.full((1, 128), 2.0, F32))
    put(C_FH, c); put(C_FH + NFQ, -sn)
    put(C_OH, jnp.where(_iota((16, 128), 1) == 0, 2.0, 0.0))
    c, sn = _cossin(fa, 8, 2 * p + 1)
    put(C_FU, c); put(C_FU + NFQ, -sn)
    k = _iota((1, NFQ), 1)
    q = k // 64
    kf = jnp.where((q == 0) | (q == 3), 1.0, -1.0) * np.float32(np.sqrt(2.0) / (2 * RB))
    c, sn = _cossin(16 * _iota((16, 1), 0) + 1, 2, 8 * (k % 64) + 2 * q + 1, kf)
    put(C_CE, c[:, :128]); put(C_CE + 128, c[:, 128:]); put(C_SO, sn[:, :128]); put(C_SO + 128, sn[:, 128:])
    r, l = _iota((128, 128), 0), _iota((128, 128), 1)
    put(C_PM, jnp.where(l == (r % 8) * 16 + r // 8, 1.0, 0.0))


def _ln(x):
    m = jnp.mean(x, axis=-1, keepdims=True)
    xc = x - m
    v = jnp.mean(xc * xc, axis=-1, keepdims=True)
    return xc * jnp.exp(-0.5 * jnp.log(v + 1e-5))


def _phi(t):
    return jnp.where(t > 0, t + 1.0, jnp.exp(t)) + 1e-6


def _dot(a, b):
    return jnp.dot(a, b, preferred_element_type=F32)


def _dot_nt(a, b):
    return lax.dot_general(a, b, (((1,), (1,)), ((), ())), preferred_element_type=F32)


def _pk(x):
    return pltpu.bitcast(x, U32)


def _upk(x):
    return pltpu.bitcast(x, BF16)


AREA = 3 * NFQ + 8
SP_ROWS = LT * AREA
RAREA = 2 * NFQ + 8
NPART = 3
PW_ROWS = (1 + NPART) * LT * RAREA
YTOK = LT * S
YA_ROWS = YTOK + 8
KVB_ROWS = LT * (S // 4) + 8
ZB_ROWS = LT * (NFQ // 2) + 8
NTICK = 64 * 3 * NR


def _kernel(q_hbm, k_hbm, v_hbm, sk_hbm, h_hbm, sd_hbm, w_hbm, wo_hbm, z_hbm,
            o_hbm,
            q_v, k_v, v_v, h_v, w_v, wo_v, o_v, sk_v, sd_v, z_sm,
            cu_s, kf_s, kl_s, hf_s, tk_s, pw, zb, ya, kvb, skb, xn_s, x_s, pq_s, pk_s, g_s, z_s,
            wqk_s, m_s, zr_s,
            sem_in, sem_o, *spb):
    su, sh = spb[:NR], spb[NR:]

    def cp_rows(src, dst, i):
        return lambda s: pltpu.make_async_copy(src.at[0, pl.ds(i * RB, RB), :], dst.at[pl.ds(i * RB, RB), :], s)

    ck = lambda i: cp_rows(k_hbm, k_v, i)
    cv = lambda i: cp_rows(v_hbm, v_v, i)
    cq = lambda i: cp_rows(q_hbm, q_v, i)
    ch = lambda i, n=1: (lambda s: pltpu.make_async_copy(h_hbm.at[:, pl.ds(i * RB, n * RB)], h_v.at[:, pl.ds(i * RB, n * RB)], s))
    cw = lambda i: (lambda s: pltpu.make_async_copy(w_hbm.at[:, pl.ds(i * D, D)], w_v.at[:, pl.ds(i * D, D)], s))
    full = lambda a, b: (lambda s: pltpu.make_async_copy(a, b, s))
    groups = [
        [full(z_hbm, z_sm)],
        [ch(0), full(sd_hbm, sd_v)],
        [full(sk_hbm, sk_v), ck(0), cv(0)],
        [cq(0)],
        [cw(1)],
        [ch(1), ck(1), cv(1)],
        [cq(1), cw(0), ch(2), ck(2), cv(2)],
        [ch(3, 2), ck(3), cv(3), cq(2), ck(4), cv(4), cq(3)],
        [ch(5, 3), ck(5), cv(5), cq(4), ck(6), cv(6), cq(5), ck(7), cv(7), cq(6), cq(7), cw(2), full(wo_hbm, wo_v)],
    ]
    for gi, g in enumerate(groups):
        for c in g:
            c(sem_in.at[gi]).start()

    ticks = []
    loads = []

    def wait(gi):
        for c in groups[gi]:
            c(sem_in.at[gi]).wait()
        del ticks[:]
        del loads[:]

    for c in range(LT):
        kf_s[c, 0:8, :] = jnp.zeros((8, 128), F32)
    g_s[...] = jnp.zeros_like(g_s)
    z_s[...] = jnp.zeros_like(z_s)

    def put_const(r, val):
        cu_s[r // 2:(r + val.shape[0]) // 2, :] = _pk(val.astype(BF16))

    _gen_consts(put_const)

    wait(0); wait(1)
    zero = z_sm[0]
    never = jnp.full((8, 128), zero, jnp.int32) != 0

    cm = lambda a, n: _upk(cu_s[a // 2:(a + n) // 2, :])
    cm2 = lambda a: jnp.concatenate([cm(a, 128), cm(a + 128, 128)], axis=1)

    def ldd(buf, r, n=8):
        return buf[pl.ds(pl.multiple_of(r + zero, 8), n), :]

    for b in spb:
        b[pl.ds(pl.multiple_of(3 * NFQ + zero, 8), 8), :] = jnp.zeros((8, 128), F32)
    pw[pl.ds(pl.multiple_of(2 * NFQ + zero, 8), 8), :] = jnp.zeros((8, 128), F32)
    kvb[pl.ds(pl.multiple_of(KVB_ROWS - 8 + zero, 8), 8), :] = jnp.zeros((8, 256), U32)
    zb[pl.ds(pl.multiple_of(ZB_ROWS - 8 + zero, 8), 8), :] = jnp.zeros((8, 256), U32)
    skb[pl.ds(pl.multiple_of(4 * LT * 8 + zero, 8), 8), :] = jnp.zeros((8, 128), F32)
    hf_s[pl.ds(pl.multiple_of(D + zero, 8), 8), :] = jnp.zeros((8, RB), U32)
    pk_s[pl.ds(pl.multiple_of(D + zero, 16), 16), :] = jnp.zeros((16, RB), BF16)
    z_s[pl.ds(pl.multiple_of(D + zero, 8), 8), :] = jnp.zeros((8, RB), F32)

    rev8 = 7 - lax.broadcasted_iota(jnp.int32, (8, 128), 0)

    def ldrev(load8, n):
        return jnp.concatenate([jnp.take_along_axis(load8(n // 8 - 1 - g), rev8, axis=0) for g in range(n // 8)], axis=0)

    def tick(val, order, load):
        for (r, c) in order:
            ticks.append(val[r * 8:(r + 1) * 8, c * 128:(c + 1) * 128])
            loads.append(float(load))

    def spread(n, cost, lo=0, hi=None):
        hi = len(ticks) if hi is None else (hi if hi >= 0 else len(ticks) + hi)
        need = n * cost
        a_, b_ = 0.0, 1e4
        for _ in range(60):
            lv = 0.5 * (a_ + b_)
            if sum(max(0.0, lv - loads[t]) for t in range(lo, hi)) < need:
                a_ = lv
            else:
                b_ = lv
        out, acc = [], 0.0
        for t in range(lo, hi):
            free = max(0.0, b_ - loads[t])
            while len(out) < n and acc + free > len(out) * cost:
                out.append(ticks[t])
            acc += free
            loads[t] = max(loads[t], b_)
        while len(out) < n:
            out.append(ticks[hi - 1])
        return out

    def sk_setup():
        skf = sk_v[...].astype(F32)
        for t in range(4):
            for c in range(LT):
                r = (t * LT + c) * 8
                skb[r:r + 8, :] = jnp.broadcast_to(skf[t:t + 1, c * 128:(c + 1) * 128], (8, 128))

    def kvrow(c, i):
        return (c * NR + i) * (HB // 2)

    def t_kv(i, win=None):
        r0 = i * RB
        kf = k_v[r0:r0 + RB, :].astype(F32)
        for c in range(LT):
            kf_s[c, 8 + r0:8 + r0 + RB, :] = kf[:, c * 128:(c + 1) * 128]
        items = [(hf, g) for hf in range(2) for g in range(HB // 32)]
        rel = spread(2 * len(items), 90.0, *win) if win is not None else None
        for k, (hf, g) in enumerate(items):
            bu, bl = r0 + HB + 32 * g, r0 + HB - 32 * (g + 1)
            vu = v_v[bu:bu + 32, hf * HW:(hf + 1) * HW].astype(F32)
            vl = v_v[bl:bl + 32, hf * HW:(hf + 1) * HW].astype(F32)
            for cl in range(2):
                c = 2 * hf + cl
                sk = [skb[(t * LT + c) * 8:(t * LT + c) * 8 + 8, :] for t in range(4)]
                if rel is not None:
                    sk = [jnp.where(never, rel[2 * k + cl], x) for x in sk]
                sk = [jnp.tile(x, (4, 1)) for x in sk]

                def kvof(b0, vf):
                    ks = (kf_s[c, 8 + b0:40 + b0, :] * sk[0] + kf_s[c, 7 + b0:39 + b0, :] * sk[1]
                          + kf_s[c, 6 + b0:38 + b0, :] * sk[2] + kf_s[c, 5 + b0:37 + b0, :] * sk[3])
                    return ks * vf[:, cl * 128:(cl + 1) * 128]
                up = kvof(bu, vu)
                lb = (c * (HB // 32) + g) * 32
                kl_s[lb:lb + 32, :] = kvof(bl, vl)
                lo = ldrev(lambda gg: kl_s[lb + gg * 8:lb + gg * 8 + 8, :], 32)
                r = kvrow(c, i) + g * 16
                kvb[r:r + 16, :] = _pk(jnp.concatenate([up + lo, up - lo], axis=1).astype(BF16))

    def put3(buf, hf, comps):
        val = jnp.stack(comps, axis=1).reshape(3 * NFQ, HW)
        for cl in range(2):
            r = (2 * hf + cl) * AREA
            buf[r:r + 3 * NFQ, :] = val[:, cl * 128:(cl + 1) * 128]

    def t_u(i):
        for hf in range(2):
            xe, xo = [jnp.concatenate([_upk(kvb[kvrow(c, i):kvrow(c, i) + HB // 2, eo * 128:(eo + 1) * 128])
                                       for c in (2 * hf, 2 * hf + 1)], axis=1) for eo in range(2)]
            ur = _dot(cm(C_FU, NFQ), xe)
            ui = _dot(cm(C_FU + NFQ, NFQ), xo)
            tick(ui, [(r, 0) for r in range(0, 32, 2)], 15)
            ur, ui = ur.reshape(16, 16, HW), ui.reshape(16, 16, HW)
            put3(su[i], hf, (ur, ui, ur + ui))

    lane = lax.broadcasted_iota(jnp.int32, (32, 128), 1)
    mirror = (128 - lane) % 128

    def t_hf(j, win=None):
        n = 32
        rel = spread(D // n, 30.0, *win) if win is not None else None
        for k in range(D // n):
            g = h_v[k * n:(k + 1) * n, j * RB:(j + 1) * RB].astype(F32)
            lo = jnp.take_along_axis(g[:, 0:128], mirror, axis=1)
            zz = jnp.zeros((8, 128), F32)
            if rel is not None:
                zz = jnp.where(never, rel[k], zz)
            up = jnp.where(lane == 0, jnp.tile(zz, (n // 8, 1)), g[:, 128:256])
            hf_s[((j % 2) * D + k * n) // 2:((j % 2) * D + (k + 1) * n) // 2, :] = _pk(
                jnp.concatenate([up + lo, up - lo], axis=1).astype(BF16))

    def t_h(j):
        for hf in range(2):
            r = ((j % 2) * D + hf * HW) // 2
            hb = _upk(hf_s[r:r + HW // 2, :])
            cen = _dot_nt(cm(C_OH, 16), h_v[hf * HW:(hf + 1) * HW, j * RB + 128:(j + 1) * RB])
            hr = _dot_nt(cm(C_FH, NFQ), hb[:, 0:128])
            hi = _dot_nt(cm(C_FH + NFQ, NFQ), hb[:, 128:256])
            tick(hi, [(r_, 0) for r_ in range(0, 32, 2)], 22)
            hr = hr.reshape(4, 4, 16, HW) + cen[None, None]
            hi = hi.reshape(4, 4, 16, HW)
            if j == 0:
                dd = sd_v[...].astype(F32).reshape(1, D)[:, hf * HW:(hf + 1) * HW] * np.float32(np.sqrt(2.0))
                hr = jnp.stack([hr[0] + dd, hr[1] - dd, hr[2] - dd, hr[3] + dd])
                hi = jnp.stack([hi[0] + dd, hi[1] + dd, hi[2] - dd, hi[3] - dd])
            hc = jnp.stack([hr[0] + hi[0], hr[1] - hi[1], hr[2] + hi[2], hr[3] - hi[3]]) * 0.5
            put3(sh[j], hf, tuple(x.reshape(16, 16, HW) for x in (hc, hr, hi)))

    def mac_slab(p, terms, first, last, c, q, t, link):
        base = c * AREA + t * 48
        lds = lambda buf, m: buf[pl.ds(pl.multiple_of(base + m * 16, 8), 16), :]
        even = q % 2 == 0
        rs = lambda slot, m: pl.ds(pl.multiple_of((slot * LT + c) * RAREA + t * 32 + m * 16, 8), 16)
        ps = 1 + p % NPART

        def chain(hm, um, acc, sign):
            for a in terms:
                tm = lds(sh[p - a], hm) * lds(su[a], um)
                acc = acc + tm if sign > 0 else acc - tm
            return acc

        if first:
            b0 = jnp.tile(jnp.where(never, link, jnp.zeros((8, 128), F32)), (2, 1))
        else:
            b0 = jnp.where(jnp.tile(never, (2, 1)), jnp.tile(link, (2, 1)), pw[rs(ps, 1), :])
        a0 = chain(1, 0, b0, -1) if even else chain(2, 0, b0, 1)
        wi = chain(0, 2, a0, 1)
        wr = chain(2 if even else 1, 1, wi - a0 if first else wi + (pw[rs(ps, 0), :] - a0), -1)
        if not last:
            pw[rs(ps, 0), :] = wr
            pw[rs(ps, 1), :] = wi
            return a0[0:8]
        if p > 0:
            qr, qi = pw[rs(0, 0), :], pw[rs(0, 1), :]
            zr, zi = (wr - qi, wi + qr) if even else (wr + qi, wi - qr)
        else:
            zr, zi = wr, wi
        if p < NR - 1:
            pw[rs(0, 0), :] = wr
            pw[rs(0, 1), :] = wi
        zb[pl.ds(pl.multiple_of(c * (NFQ // 2) + t * 8, 8), 8), :] = _pk(jnp.concatenate([zr, zi], axis=1).astype(BF16))
        return a0[0:8]

    done = [[] for _ in range(NR)]
    ntk = [0]

    def mac(p, terms=None, win=None):
        if terms is None:
            terms = [a for a in list(range(1, p)) + ([0, p] if p > 0 else [0]) if a not in done[p]]
        first = not done[p]
        done[p] += list(terms)
        last = len(done[p]) == p + 1
        base = ntk[0]
        if win is not None:
            ntk[0] += 64
            for k, val in enumerate(spread(64, 12.0 * len(terms) + 10, *win)):
                tk_s[(base + k) * 8:(base + k + 1) * 8, :] = val
        link = jnp.zeros((8, 128), F32)
        for c in range(LT):
            for q in range(4):
                def body(tt, carry):
                    if win is not None:
                        carry = tk_s[pl.ds(pl.multiple_of((base + c * 16 + q * 4 + tt) * 8, 8), 8), :]
                    return mac_slab(p, terms, first, last, c, q, q * 4 + tt, carry)
                link = lax.fori_loop(0, 4, body, link, unroll=True)

    def t_inv(i):
        for hf in range(2):
            zr, zi = [jnp.concatenate([_upk(zb[c * (NFQ // 2):(c + 1) * (NFQ // 2), m * 128:(m + 1) * 128])
                                       for c in (2 * hf, 2 * hf + 1)], axis=1) for m in range(2)]
            e = _dot(cm2(C_CE), zr)
            o = _dot(cm2(C_SO), zi)
            tick(o, [(r, 1) for r in range(16)], 8)
            hi_, lo_ = e - o, e + o
            for cl in range(2):
                r = (2 * hf + cl) * S + i * RB
                ya[r:r + HB, :] = lo_[:, cl * 128:(cl + 1) * 128]
                ya[r + HB:r + RB, :] = hi_[:, cl * 128:(cl + 1) * 128]

    def get_y(r0, n, chained):
        ld = (lambda r, k: ldd(ya, r, k)) if chained else (lambda r, k: ya[r:r + k, :])
        blk, off = r0 // RB, r0 % RB
        cols = []
        for c in range(LT):
            b = c * S + blk * RB
            parts = []
            nl = max(0, min(off + n, HB) - off)
            if nl:
                s0 = b + HB - off - nl
                parts.append(ldrev(lambda gg: ld(s0 + gg * 8, 8), nl))
            if n - nl:
                parts.append(ld(b + off + nl, n - nl))
            cols.append(parts[0] if len(parts) == 1 else jnp.concatenate(parts, axis=0))
        return jnp.concatenate(cols, axis=1)

    def ln_rows(r0, n, x, chained):
        x = x + _ln(x) * get_y(r0, n, chained)
        x_s[r0:r0 + n, :] = x
        xnf = _ln(x)
        xn_s[r0 // 2:(r0 + n) // 2, :] = _pk(xnf.astype(BF16))
        if chained:
            tok = xnf[0:8, 0:128]
            for g in range(1, n // 8):
                tok = tok + xnf[g * 8:(g + 1) * 8, (g % LT) * 128:(g % LT + 1) * 128]
            ya[YTOK:YTOK + 8, :] = tok

    def t_ln(i, sizes=(64,) * 4):
        r0 = i * RB
        for n in sizes:
            ln_rows(r0, n, q_v[r0:r0 + n, :].astype(F32), True)
            r0 += n

    def ln_chain(i, x):
        ln_rows(i * RB, RB, x, False)

    def xn(i):
        return _upk(xn_s[i * RB // 2:(i + 1) * RB // 2, :])

    def t_q(i):
        r0 = i * RB
        pq_s[r0:r0 + RB, :] = _dot_nt(xn(i), _upk(wqk_s[0:D // 2, :])).astype(BF16)

    def q_half(i, h):
        r0 = i * RB
        qs = []
        for n in (2 * h, 2 * h + 1):
            qq = _dot_nt(xn(i), _upk(wqk_s[n * 64:(n + 1) * 64, :]))
            tick(qq, [(r, 0) for r in range(0, 32, 2)], 7)
            qs.append(qq)
        pq_s[r0:r0 + RB, h * HW:(h + 1) * HW] = jnp.concatenate(qs, axis=1).astype(BF16)

    def kgp(i, mem=True):
        st = {}

        def kt():
            kt = _dot_nt(_upk(wqk_s[D // 2:D, :]), xn(i))
            tick(kt, [(r, c) for c in range(2) for r in range(0, D // 8, 2)], 19)
            pkt = _phi(kt)
            z_s[0:D, :] += pkt
            if mem:
                for c in range(2):
                    pk_s[0:D, c * 128:(c + 1) * 128] = pkt[:, c * 128:(c + 1) * 128].astype(BF16)
            else:
                st[0] = pkt.astype(BF16)

        def gm():
            gg = _dot(pk_s[0:D, :] if mem else st[0], xn(i))
            tick(gg, [(r, c) for c in (1, 3) for r in range(0, D // 8, 2)], 8)
            g_s[...] += gg
        return [kt, gm]

    def wprep(part):
        for gp in range(2):
            for hf in range(2):
                blk = [_dot_nt(cm(C_PM, 128), w_v[hf * HW:(hf + 1) * HW, part * D + g * 128: part * D + (g + 1) * 128])
                       for g in (2 * gp, 2 * gp + 1)]
                tick(blk[1], [(r, 0) for r in range(0, 16, 2)], 8)
                rows = jnp.stack([x.reshape(16, 8, HW) for x in blk], axis=1).reshape(256, HW)
                for e in range(16):
                    r = part * (D // 2) + e * 16 + gp * 8
                    wqk_s[r:r + 8, hf * HW:(hf + 1) * HW] = _pk(rows[e * 16:(e + 1) * 16].astype(BF16))

    def finalize(last, fill):
        zt = (z_s[0:D, 0:128] + z_s[0:D, 128:256]).T
        zr_s[...] = jnp.broadcast_to(jnp.sum(zt, axis=0, keepdims=True), (8, D))
        rr = lax.broadcasted_iota(jnp.int32, (128, 128), 0) % 8
        cc_ = lax.broadcasted_iota(jnp.int32, (128, 128), 1) // DH
        mask = rr == cc_
        fill[0]()
        kvs = []
        for g in range(4):
            gg = jnp.concatenate([g_s[e * 32 + g * 8: e * 32 + g * 8 + 8, :] for e in range(16)], axis=0).astype(BF16)
            wv = w_v[:, 2 * D + g * 128: 2 * D + (g + 1) * 128]
            kvs.append(jnp.where(mask, _dot(gg, wv), 0.0).astype(BF16))
        fill[1]()
        ms = [_dot(kvs[g], wo_v[g * 128:(g + 1) * 128, :]) for g in range(4)]
        for e in range(16):
            rows = jnp.concatenate([ms[g][e * 8:(e + 1) * 8] for g in range(4)], axis=0)
            m_s[e * 16:(e + 1) * 16, :] = _pk(rows.astype(BF16))
        fill[2]()
        if not last:
            g_s[...] = jnp.zeros_like(g_s)
            z_s[0:D, :] = jnp.zeros((D, RB), F32)

    def q_cols(i, n0, n1):
        r0 = i * RB
        pq_s[r0:r0 + RB, n0:n1] = _dot_nt(xn(i), _upk(wqk_s[n0 // 2:n1 // 2, :])).astype(BF16)

    def q_fill(i):
        return [functools.partial(q_cols, i, 0, 256), functools.partial(q_cols, i, 256, 384), functools.partial(q_cols, i, 384, 512)]

    def s5_att(i, r0=None, n=RB):
        r0 = i * RB if r0 is None else r0
        pq = _phi(pq_s[r0:r0 + n, :].astype(F32))
        t = pq * zr_s[0:1, :]
        t = (t[:, 0:128] + t[:, 128:256]) + (t[:, 256:384] + t[:, 384:512])
        t = t + pltpu.roll(t, 64, 1)
        t = t + pltpu.roll(t, 32, 1)
        den = t + 1e-6
        r = pl.reciprocal(den, approx=True)
        r = r * (2.0 - den * r)
        a = (pq * jnp.concatenate([r] * LT, axis=1)).astype(BF16)
        return x_s[r0:r0 + n, :] + _dot(a, _upk(m_s[...]))

    F = functools.partial
    Q = lambda i, *hs: [F(q_half, i, h) for h in (hs or (0, 1))]

    def run(ts):
        for t in ts:
            t()

    def region(r, pre, post, bwork=(), nxt=True, ln=(32,) * 8, lnt=170, tail=TAIL):
        run(pre)
        mac(r, None, (0, -4))
        t_inv(r)
        t1 = len(ticks)
        run(post)
        for t in range(t1 - 8, min(len(ticks), t1 - 8 + lnt)):
            loads[t] += LN_OPS / lnt
        if nxt:
            t_kv(r + 1, (0, -10))
            t_hf(r + 1, (0, -10))
            t_h(r + 1); t_u(r + 1)
        for p_, terms in bwork:
            mac(p_, terms, (0, -tail))
        t_ln(r, ln)

    t_hf(0); t_h(0)
    wait(2)
    sk_setup(); t_kv(0)
    wait(3)
    t_u(0); mac(0); t_inv(0)
    wait(4)
    kg = kgp(0)
    wprep(1); t_ln(0, (256,)); kg[0]()
    wait(5)
    kg[1](); t_hf(1, (0, 24)); t_kv(1, (0, -16)); t_h(1); t_u(1)
    wait(6)
    region(1, [F(wprep, 0)], Q(0), [(2, [1])], ln=(64,) * 4, lnt=90)
    for r in range(2, NR):
        if r in (2, 4):
            wait(7 if r == 2 else 8)
        del ticks[:]; del loads[:]
        kg = kgp(r - 1)
        bw = [(r + 1, list(range(1, r + 1)))] if r + 1 < NR else []
        if r + 1 < NR:
            region(r, Q(r - 1), kg, bw, tail=TAIL if r == 3 else 1)
        else:
            region(r, Q(r - 1, 0), kg + Q(r - 1, 1), nxt=False, ln=(64,) * 4)
    run(kgp(7))
    finalize(False, q_fill(NR - 1))

    ln_chain(0, s5_att(0))
    for i in range(NR):
        if i + 1 < NR:
            x = s5_att(i + 1)
        run(kgp(i, False))
        if i + 1 < NR:
            ln_chain(i + 1, x)
            t_q(i)
    finalize(True, q_fill(NR - 1))

    chunks = [(i * RB, RB) for i in range(NR - 1)] + [(S - RB, 128), (S - 128, 128)]
    cps = []
    for r0, n in chunks:
        o_v[r0:r0 + n, :] = s5_att(0, r0, n).astype(BF16)
        cps.append(pltpu.make_async_copy(o_v.at[pl.ds(r0, n), :], o_hbm.at[0, pl.ds(r0, n), :], sem_o.at[0]))
        cps[-1].start()
    for cp in cps:
        cp.wait()


@jax.jit
def pallas_interleave_layers__ssm_conv_h3__linear_attn_block__prompt_kernel(
        A_q, A_k, A_v, A_shift_k, A_ssm_k, A_ssm_D, B_x, B_wqkv, B_wo):
    z = jnp.asarray(np.zeros((8,), np.int32))
    any_spec = pl.BlockSpec(memory_space=pl.ANY)
    return pl.pallas_call(
        _kernel,
        out_shape=jax.ShapeDtypeStruct((1, S, D), BF16),
        in_specs=[any_spec] * 9,
        out_specs=any_spec,
        scratch_shapes=[
            pltpu.VMEM((S, D), BF16),
            pltpu.VMEM((S, D), BF16),
            pltpu.VMEM((S, D), BF16),
            pltpu.VMEM((D, S), BF16),
            pltpu.VMEM((D, 3 * D), BF16),
            pltpu.VMEM((D, D), BF16),
            pltpu.VMEM((S, D), BF16),
            pltpu.VMEM((4, D), BF16),
            pltpu.VMEM((D,), BF16),
            pltpu.SMEM((8,), jnp.int32),
            pltpu.VMEM((C_ROWS // 2, 128), U32),
            pltpu.VMEM((LT, 8 + S, 128), F32),
            pltpu.VMEM((LT * HB, 128), F32),
            pltpu.VMEM((D + 8, RB), U32),
            pltpu.VMEM((NTICK * 8, 128), F32),
            pltpu.VMEM((PW_ROWS, 128), F32),
            pltpu.VMEM((ZB_ROWS, 256), U32),
            pltpu.VMEM((YA_ROWS, 128), F32),
            pltpu.VMEM((KVB_ROWS, 256), U32),
            pltpu.VMEM((4 * LT * 8 + 8, 128), F32),
            pltpu.VMEM((S // 2, D), U32),
            pltpu.VMEM((S, D), F32),
            pltpu.VMEM((S, D), BF16),
            pltpu.VMEM((D + 16, RB), BF16),
            pltpu.VMEM((D, D), F32),
            pltpu.VMEM((D + 8, RB), F32),
            pltpu.VMEM((D, D), U32),
            pltpu.VMEM((D // 2, D), U32),
            pltpu.VMEM((8, D), F32),
            pltpu.SemaphoreType.DMA((9,)),
            pltpu.SemaphoreType.DMA((1,)),
        ] + [pltpu.VMEM((SP_ROWS, 128), F32)] * (2 * NR),
        compiler_params=pltpu.CompilerParams(vmem_limit_bytes=110 * 1024 * 1024),
    )(A_q, A_k, A_v, A_shift_k.T, A_ssm_k, A_ssm_D, B_wqkv, B_wo, z)
```

```python
import functools
import numpy as np
import jax
import jax.numpy as jnp
from jax import lax
import jax.experimental.pallas as pl
import jax.experimental.pallas.tpu as pltpu

S, D = 2048, 512
RB = 256
NR = S // RB
NFQ = 256
HB = RB // 2
DH = 16
LT = D // 128
HW = D // 2
F32 = jnp.float32
BF16 = jnp.bfloat16
U32 = jnp.uint32
TAIL = 14
LN_OPS = 1900.0


C_FH, C_OH, C_FU, C_CE, C_SO, C_PM, C_ROWS = 0, 512, 528, 1040, 1296, 1552, 1680


def _iota(shape, d):
    return lax.broadcasted_iota(jnp.int32, shape, d)


def _cossin(row_a, row_step, col, scale=None):
    nt, w = row_a.shape[0], col.shape[1]
    ang = lambda ph: (ph & 2047).astype(F32) * np.float32(np.pi / 1024.0)
    ta = ang(row_a * col)
    tb = ang(_iota((8, w), 0) * row_step * col)
    ca, sa, cb, sb = jnp.cos(ta), jnp.sin(ta), jnp.cos(tb), jnp.sin(tb)
    if scale is not None:
        cb, sb = cb * scale, sb * scale
    cs = [ca[t:t + 1] * cb - sa[t:t + 1] * sb for t in range(nt)]
    sn = [sa[t:t + 1] * cb + ca[t:t + 1] * sb for t in range(nt)]
    return jnp.concatenate(cs, axis=0), jnp.concatenate(sn, axis=0)


def _gen_consts(put):
    t = _iota((32, 1), 0)
    fa = 64 * (t % 8) + 2 * (t // 8) + 1
    p = _iota((1, 128), 1)
    c, sn = _cossin(fa, 8, jnp.where(p == 0, 2 * HB, 2 * p), jnp.full((1, 128), 2.0, F32))
    put(C_FH, c); put(C_FH + NFQ, -sn)
    put(C_OH, jnp.where(_iota((16, 128), 1) == 0, 2.0, 0.0))
    c, sn = _cossin(fa, 8, 2 * p + 1)
    put(C_FU, c); put(C_FU + NFQ, -sn)
    k = _iota((1, NFQ), 1)
    q = k // 64
    kf = jnp.where((q == 0) | (q == 3), 1.0, -1.0) * np.float32(np.sqrt(2.0) / (2 * RB))
    c, sn = _cossin(16 * _iota((16, 1), 0) + 1, 2, 8 * (k % 64) + 2 * q + 1, kf)
    put(C_CE, c[:, :128]); put(C_CE + 128, c[:, 128:]); put(C_SO, sn[:, :128]); put(C_SO + 128, sn[:, 128:])
    r, l = _iota((128, 128), 0), _iota((128, 128), 1)
    put(C_PM, jnp.where(l == (r % 8) * 16 + r // 8, 1.0, 0.0))


def _ln(x):
    m = jnp.mean(x, axis=-1, keepdims=True)
    xc = x - m
    v = jnp.mean(xc * xc, axis=-1, keepdims=True)
    return xc * jnp.exp(-0.5 * jnp.log(v + 1e-5))


def _phi(t):
    return jnp.where(t > 0, t + 1.0, jnp.exp(t)) + 1e-6


def _dot(a, b):
    return jnp.dot(a, b, preferred_element_type=F32)


def _dot_nt(a, b):
    return lax.dot_general(a, b, (((1,), (1,)), ((), ())), preferred_element_type=F32)


def _pk(x):
    return pltpu.bitcast(x, U32)


def _upk(x):
    return pltpu.bitcast(x, BF16)


AREA = 3 * NFQ + 8
SP_ROWS = LT * AREA
RAREA = 2 * NFQ + 8
NPART = 3
PW_ROWS = (1 + NPART) * LT * RAREA
YTOK = LT * S
YA_ROWS = YTOK + 8
KVB_ROWS = LT * (S // 4) + 8
ZB_ROWS = LT * (NFQ // 2) + 8
NTICK = 64 * 3 * NR


def _kernel(q_hbm, k_hbm, v_hbm, sk_hbm, h_hbm, sd_hbm, w_hbm, wo_hbm, z_hbm,
            o_hbm,
            q_v, k_v, v_v, h_v, w_v, wo_v, o_v, sk_v, sd_v, z_sm,
            cu_s, kf_s, kl_s, hf_s, tk_s, pw, zb, ya, kvb, skb, xn_s, x_s, pq_s, pk_s, g_s, z_s,
            wqk_s, m_s, zr_s, xa_s, xb_s, x2_s, q2_s,
            sem_in, sem_o, *spb):
    su, sh = spb[:NR], spb[NR:]

    def cp_rows(src, dst, i):
        return lambda s: pltpu.make_async_copy(src.at[0, pl.ds(i * RB, RB), :], dst.at[pl.ds(i * RB, RB), :], s)

    ck = lambda i: cp_rows(k_hbm, k_v, i)
    cv = lambda i: cp_rows(v_hbm, v_v, i)
    cq = lambda i: cp_rows(q_hbm, q_v, i)
    ch = lambda i, n=1: (lambda s: pltpu.make_async_copy(h_hbm.at[:, pl.ds(i * RB, n * RB)], h_v.at[:, pl.ds(i * RB, n * RB)], s))
    cw = lambda i: (lambda s: pltpu.make_async_copy(w_hbm.at[:, pl.ds(i * D, D)], w_v.at[:, pl.ds(i * D, D)], s))
    full = lambda a, b: (lambda s: pltpu.make_async_copy(a, b, s))
    groups = [
        [full(z_hbm, z_sm)],
        [ch(0), full(sd_hbm, sd_v)],
        [full(sk_hbm, sk_v), ck(0), cv(0)],
        [cq(0)],
        [cw(1)],
        [ch(1), ck(1), cv(1)],
        [cq(1), cw(0), ch(2), ck(2), cv(2)],
        [ch(3), ck(3), cv(3), cq(2)],
        [ch(4, 2), ck(4), cv(4), cq(3), ck(5), cv(5), cq(4)],
        [ch(6, 2), ck(6), cv(6), cq(5), ck(7), cv(7), cq(6), cq(7), cw(2), full(wo_hbm, wo_v)],
    ]
    for gi, g in enumerate(groups):
        for c in g:
            c(sem_in.at[gi]).start()

    ticks = []
    loads = []

    def wait(gi):
        for c in groups[gi]:
            c(sem_in.at[gi]).wait()
        del ticks[:]
        del loads[:]

    for c in range(LT):
        kf_s[c, 0:8, :] = jnp.zeros((8, 128), F32)

    def put_const(r, val):
        cu_s[r // 2:(r + val.shape[0]) // 2, :] = _pk(val.astype(BF16))

    _gen_consts(put_const)

    wait(0); wait(1)
    zero = z_sm[0]
    never = jnp.full((8, 128), zero, jnp.int32) != 0

    cm = lambda a, n: _upk(cu_s[a // 2:(a + n) // 2, :])
    cm2 = lambda a: jnp.concatenate([cm(a, 128), cm(a + 128, 128)], axis=1)

    def ldd(buf, r, n=8):
        return buf[pl.ds(pl.multiple_of(r + zero, 8), n), :]

    for b in spb:
        b[pl.ds(pl.multiple_of(3 * NFQ + zero, 8), 8), :] = jnp.zeros((8, 128), F32)
    pw[pl.ds(pl.multiple_of(2 * NFQ + zero, 8), 8), :] = jnp.zeros((8, 128), F32)
    kvb[pl.ds(pl.multiple_of(KVB_ROWS - 8 + zero, 8), 8), :] = jnp.zeros((8, 256), U32)
    zb[pl.ds(pl.multiple_of(ZB_ROWS - 8 + zero, 8), 8), :] = jnp.zeros((8, 256), U32)
    skb[pl.ds(pl.multiple_of(4 * LT * 8 + zero, 8), 8), :] = jnp.zeros((8, 128), F32)
    hf_s[pl.ds(pl.multiple_of(D + zero, 8), 8), :] = jnp.zeros((8, RB), U32)
    pk_s[pl.ds(pl.multiple_of(D + zero, 16), 16), :] = jnp.zeros((16, RB), BF16)
    z_s[pl.ds(pl.multiple_of(D + zero, 8), 8), :] = jnp.zeros((8, RB), F32)

    rev8 = 7 - lax.broadcasted_iota(jnp.int32, (8, 128), 0)

    def ldrev(load8, n):
        return jnp.concatenate([jnp.take_along_axis(load8(n // 8 - 1 - g), rev8, axis=0) for g in range(n // 8)], axis=0)

    def tick(val, order, load):
        for (r, c) in order:
            ticks.append(val[r * 8:(r + 1) * 8, c * 128:(c + 1) * 128])
            loads.append(float(load))

    def spread(n, cost, lo=0, hi=None):
        hi = len(ticks) if hi is None else (hi if hi >= 0 else len(ticks) + hi)
        need = n * cost
        a_, b_ = 0.0, 1e4
        for _ in range(60):
            lv = 0.5 * (a_ + b_)
            if sum(max(0.0, lv - loads[t]) for t in range(lo, hi)) < need:
                a_ = lv
            else:
                b_ = lv
        out, acc = [], 0.0
        for t in range(lo, hi):
            free = max(0.0, b_ - loads[t])
            while len(out) < n and acc + free > len(out) * cost:
                out.append(ticks[t])
            acc += free
            loads[t] = max(loads[t], b_)
        while len(out) < n:
            out.append(ticks[hi - 1])
        return out

    def sk_setup():
        skf = sk_v[...].astype(F32)
        for t in range(4):
            for c in range(LT):
                r = (t * LT + c) * 8
                skb[r:r + 8, :] = jnp.broadcast_to(skf[t:t + 1, c * 128:(c + 1) * 128], (8, 128))

    def kvrow(c, i):
        return (c * NR + i) * (HB // 2)

    def t_kv(i, win=None):
        r0 = i * RB
        kf = k_v[r0:r0 + RB, :].astype(F32)
        for c in range(LT):
            kf_s[c, 8 + r0:8 + r0 + RB, :] = kf[:, c * 128:(c + 1) * 128]
        items = [(hf, g) for hf in range(2) for g in range(HB // 32)]
        rel = spread(2 * len(items), 90.0, *win) if win is not None else None
        for k, (hf, g) in enumerate(items):
            bu, bl = r0 + HB + 32 * g, r0 + HB - 32 * (g + 1)
            vu = v_v[bu:bu + 32, hf * HW:(hf + 1) * HW].astype(F32)
            vl = v_v[bl:bl + 32, hf * HW:(hf + 1) * HW].astype(F32)
            for cl in range(2):
                c = 2 * hf + cl
                sk = [skb[(t * LT + c) * 8:(t * LT + c) * 8 + 8, :] for t in range(4)]
                if rel is not None:
                    sk = [jnp.where(never, rel[2 * k + cl], x) for x in sk]
                sk = [jnp.tile(x, (4, 1)) for x in sk]

                def kvof(b0, vf):
                    ks = (kf_s[c, 8 + b0:40 + b0, :] * sk[0] + kf_s[c, 7 + b0:39 + b0, :] * sk[1]
                          + kf_s[c, 6 + b0:38 + b0, :] * sk[2] + kf_s[c, 5 + b0:37 + b0, :] * sk[3])
                    return ks * vf[:, cl * 128:(cl + 1) * 128]
                up = kvof(bu, vu)
                lb = (c * (HB // 32) + g) * 32
                kl_s[lb:lb + 32, :] = kvof(bl, vl)
                lo = ldrev(lambda gg: kl_s[lb + gg * 8:lb + gg * 8 + 8, :], 32)
                r = kvrow(c, i) + g * 16
                kvb[r:r + 16, :] = _pk(jnp.concatenate([up + lo, up - lo], axis=1).astype(BF16))

    def put3(buf, hf, comps):
        val = jnp.stack(comps, axis=1).reshape(3 * NFQ, HW)
        for cl in range(2):
            r = (2 * hf + cl) * AREA
            buf[r:r + 3 * NFQ, :] = val[:, cl * 128:(cl + 1) * 128]

    def t_u(i):
        for hf in range(2):
            xe, xo = [jnp.concatenate([_upk(kvb[kvrow(c, i):kvrow(c, i) + HB // 2, eo * 128:(eo + 1) * 128])
                                       for c in (2 * hf, 2 * hf + 1)], axis=1) for eo in range(2)]
            ur = _dot(cm(C_FU, NFQ), xe)
            ui = _dot(cm(C_FU + NFQ, NFQ), xo)
            tick(ui, [(r, 0) for r in range(0, 32, 2)], 15)
            ur, ui = ur.reshape(16, 16, HW), ui.reshape(16, 16, HW)
            put3(su[i], hf, (ur, ui, ur + ui))

    lane = lax.broadcasted_iota(jnp.int32, (32, 128), 1)
    mirror = (128 - lane) % 128

    def t_hf(j, win=None):
        n = 32
        rel = spread(D // n, 30.0, *win) if win is not None else None
        for k in range(D // n):
            g = h_v[k * n:(k + 1) * n, j * RB:(j + 1) * RB].astype(F32)
            lo = jnp.take_along_axis(g[:, 0:128], mirror, axis=1)
            zz = jnp.zeros((8, 128), F32)
            if rel is not None:
                zz = jnp.where(never, rel[k], zz)
            up = jnp.where(lane == 0, jnp.tile(zz, (n // 8, 1)), g[:, 128:256])
            hf_s[((j % 2) * D + k * n) // 2:((j % 2) * D + (k + 1) * n) // 2, :] = _pk(
                jnp.concatenate([up + lo, up - lo], axis=1).astype(BF16))

    def t_h(j):
        for hf in range(2):
            r = ((j % 2) * D + hf * HW) // 2
            hb = _upk(hf_s[r:r + HW // 2, :])
            cen = _dot_nt(cm(C_OH, 16), h_v[hf * HW:(hf + 1) * HW, j * RB + 128:(j + 1) * RB])
            hr = _dot_nt(cm(C_FH, NFQ), hb[:, 0:128])
            hi = _dot_nt(cm(C_FH + NFQ, NFQ), hb[:, 128:256])
            tick(hi, [(r_, 0) for r_ in range(0, 32, 2)], 22)
            hr = hr.reshape(4, 4, 16, HW) + cen[None, None]
            hi = hi.reshape(4, 4, 16, HW)
            if j == 0:
                dd = sd_v[...].astype(F32).reshape(1, D)[:, hf * HW:(hf + 1) * HW] * np.float32(np.sqrt(2.0))
                hr = jnp.stack([hr[0] + dd, hr[1] - dd, hr[2] - dd, hr[3] + dd])
                hi = jnp.stack([hi[0] + dd, hi[1] + dd, hi[2] - dd, hi[3] - dd])
            hc = jnp.stack([hr[0] + hi[0], hr[1] - hi[1], hr[2] + hi[2], hr[3] - hi[3]]) * 0.5
            put3(sh[j], hf, tuple(x.reshape(16, 16, HW) for x in (hc, hr, hi)))

    def mac_slab(p, terms, first, last, c, q, t, link):
        base = c * AREA + t * 48
        lds = lambda buf, m: buf[pl.ds(pl.multiple_of(base + m * 16, 8), 16), :]
        even = q % 2 == 0
        rs = lambda slot, m: pl.ds(pl.multiple_of((slot * LT + c) * RAREA + t * 32 + m * 16, 8), 16)
        ps = 1 + p % NPART

        def chain(hm, um, acc, sign):
            for a in terms:
                tm = lds(sh[p - a], hm) * lds(su[a], um)
                acc = acc + tm if sign > 0 else acc - tm
            return acc

        if first:
            b0 = jnp.tile(jnp.where(never, link, jnp.zeros((8, 128), F32)), (2, 1))
        else:
            b0 = jnp.where(jnp.tile(never, (2, 1)), jnp.tile(link, (2, 1)), pw[rs(ps, 1), :])
        a0 = chain(1, 0, b0, -1) if even else chain(2, 0, b0, 1)
        wi = chain(0, 2, a0, 1)
        wr = chain(2 if even else 1, 1, wi - a0 if first else wi + (pw[rs(ps, 0), :] - a0), -1)
        if not last:
            pw[rs(ps, 0), :] = wr
            pw[rs(ps, 1), :] = wi
            return
        if p > 0:
            qr, qi = pw[rs(0, 0), :], pw[rs(0, 1), :]
            zr, zi = (wr - qi, wi + qr) if even else (wr + qi, wi - qr)
        else:
            zr, zi = wr, wi
        if p < NR - 1:
            pw[rs(0, 0), :] = wr
            pw[rs(0, 1), :] = wi
        zb[pl.ds(pl.multiple_of(c * (NFQ // 2) + t * 8, 8), 8), :] = _pk(jnp.concatenate([zr, zi], axis=1).astype(BF16))

    done = [[] for _ in range(NR)]
    ntk = [0]

    def mac(p, terms=None, win=None):
        if terms is None:
            terms = [a for a in list(range(1, p)) + ([0, p] if p > 0 else [0]) if a not in done[p]]
        first = not done[p]
        done[p] += list(terms)
        last = len(done[p]) == p + 1
        base = ntk[0]
        if win is not None:
            ntk[0] += 64
            for k, val in enumerate(spread(64, 12.0 * len(terms) + 10, *win)):
                tk_s[(base + k) * 8:(base + k + 1) * 8, :] = val
        link = jnp.zeros((8, 128), F32)
        for c in range(LT):
            for q in range(4):
                def body(tt, carry):
                    if win is not None:
                        carry = tk_s[pl.ds(pl.multiple_of((base + c * 16 + q * 4 + tt) * 8, 8), 8), :]
                    mac_slab(p, terms, first, last, c, q, q * 4 + tt, carry)
                    return carry
                lax.fori_loop(0, 4, body, link, unroll=True)

    def t_inv(i):
        for c in range(LT):
            zz = _upk(zb[c * (NFQ // 2):(c + 1) * (NFQ // 2), :])
            e = _dot(cm2(C_CE), zz[:, 0:128])
            o = _dot(cm2(C_SO), zz[:, 128:256])
            tick(o, [(r, 0) for r in range(0, 16, 2)], 8)
            r = c * S + i * RB
            ya[r:r + HB, :] = e + o
            ya[r + HB:r + RB, :] = e - o

    def get_y(r0, n, chained):
        ld = (lambda r, k: ldd(ya, r, k)) if chained else (lambda r, k: ya[r:r + k, :])
        blk, off = r0 // RB, r0 % RB
        cols = []
        for c in range(LT):
            b = c * S + blk * RB
            parts = []
            nl = max(0, min(off + n, HB) - off)
            if nl:
                s0 = b + HB - off - nl
                parts.append(ldrev(lambda gg: ld(s0 + gg * 8, 8), nl))
            if n - nl:
                parts.append(ld(b + off + nl, n - nl))
            cols.append(parts[0] if len(parts) == 1 else jnp.concatenate(parts, axis=0))
        return jnp.concatenate(cols, axis=1)

    def ln_rows(r0, n, x, chained, ln1=None):
        x = x + (_ln(x) if ln1 is None else ln1) * get_y(r0, n, chained)
        x_s[r0:r0 + n, :] = x
        xnf = _ln(x)
        xn_s[r0 // 2:(r0 + n) // 2, :] = _pk(xnf.astype(BF16))
        if chained:
            tok = xnf[0:8, 0:128]
            for g in range(1, n // 8):
                tok = tok + xnf[g * 8:(g + 1) * 8, (g % LT) * 128:(g % LT + 1) * 128]
            ya[YTOK:YTOK + 8, :] = tok

    def t_ln(i, sizes=(64,) * 4):
        r0 = i * RB
        for n in sizes:
            ln_rows(r0, n, q_v[r0:r0 + n, :].astype(F32), True)
            r0 += n

    def xn(i):
        return _upk(xn_s[i * RB // 2:(i + 1) * RB // 2, :])

    def q_half(i, h):
        r0 = i * RB
        qs = []
        for n in (2 * h, 2 * h + 1):
            qq = _dot_nt(xn(i), _upk(wqk_s[n * 64:(n + 1) * 64, :]))
            tick(qq, [(r, 0) for r in range(0, 32, 2)], 7)
            qs.append(qq)
        pq_s[r0:r0 + RB, h * HW:(h + 1) * HW] = jnp.concatenate(qs, axis=1).astype(BF16)

    def kgp(i):
        def kt():
            kt = _dot_nt(_upk(wqk_s[D // 2:D, :]), xn(i))
            tick(kt, [(r, c) for c in range(2) for r in range(0, D // 8, 2)], 19)
            pkt = _phi(kt)
            z_s[0:D, :] = pkt if i == 0 else z_s[0:D, :] + pkt
            for c in range(2):
                pk_s[0:D, c * 128:(c + 1) * 128] = pkt[:, c * 128:(c + 1) * 128].astype(BF16)

        def gm():
            gg = _dot(pk_s[0:D, :], xn(i))
            tick(gg, [(r, c) for c in (1, 3) for r in range(0, D // 8, 2)], 8)
            g_s[...] = gg if i == 0 else g_s[...] + gg
        return [kt, gm]

    def wprep(part):
        for gp in range(2):
            for hf in range(2):
                blk = [_dot_nt(cm(C_PM, 128), w_v[hf * HW:(hf + 1) * HW, part * D + g * 128: part * D + (g + 1) * 128])
                       for g in (2 * gp, 2 * gp + 1)]
                tick(blk[1], [(r, 0) for r in range(0, 16, 2)], 8)
                rows = jnp.stack([x.reshape(16, 8, HW) for x in blk], axis=1).reshape(256, HW)
                for e in range(16):
                    r = part * (D // 2) + e * 16 + gp * 8
                    wqk_s[r:r + 8, hf * HW:(hf + 1) * HW] = _pk(rows[e * 16:(e + 1) * 16].astype(BF16))

    def finalize(fill):
        zt = (z_s[0:D, 0:128] + z_s[0:D, 128:256]).T
        zr_s[...] = jnp.broadcast_to(jnp.sum(zt, axis=0, keepdims=True), (8, D))
        rr = lax.broadcasted_iota(jnp.int32, (128, 128), 0) % 8
        cc_ = lax.broadcasted_iota(jnp.int32, (128, 128), 1) // DH
        mask = rr == cc_
        fill[0]()
        kvs = []
        for g in range(4):
            gg = jnp.concatenate([g_s[e * 32 + g * 8: e * 32 + g * 8 + 8, :] for e in range(16)], axis=0).astype(BF16)
            wv = w_v[:, 2 * D + g * 128: 2 * D + (g + 1) * 128]
            kvs.append(jnp.where(mask, _dot(gg, wv), 0.0).astype(BF16))
        fill[1]()
        ms = [_dot(kvs[g], wo_v[g * 128:(g + 1) * 128, :]) for g in range(4)]
        for e in range(16):
            rows = jnp.concatenate([ms[g][e * 8:(e + 1) * 8] for g in range(4)], axis=0)
            m_s[e * 16:(e + 1) * 16, :] = _pk(rows.astype(BF16))
        fill[2]()

    def q_cols(i, n0, n1):
        r0 = i * RB
        pq_s[r0:r0 + RB, n0:n1] = _dot_nt(xn(i), _upk(wqk_s[n0 // 2:n1 // 2, :])).astype(BF16)

    def q_fill(i):
        return [functools.partial(q_cols, i, 0, 256), functools.partial(q_cols, i, 256, 384), functools.partial(q_cols, i, 384, 512)]

    F = functools.partial
    Q = lambda i, *hs: [F(q_half, i, h) for h in (hs or (0, 1))]

    def run(ts):
        for t in ts:
            t()

    def region(r, pre, post, bwork=(), nxt=True, ln=(32,) * 8, lnt=170, tail=TAIL):
        run(pre)
        mac(r, None, (0, -4))
        t_inv(r)
        t1 = len(ticks)
        run(post)
        for t in range(t1 - 8, min(len(ticks), t1 - 8 + lnt)):
            loads[t] += LN_OPS / lnt
        if nxt:
            t_kv(r + 1, (0, -10))
            t_hf(r + 1, (0, -10))
            t_h(r + 1); t_u(r + 1)
        for p_, terms in bwork:
            mac(p_, terms, (0, -tail))
        t_ln(r, ln)

    t_hf(0); t_h(0)
    wait(2)
    sk_setup(); t_kv(0)
    wait(3)
    t_u(0); mac(0); t_inv(0)
    x_s[0:RB, :] = _ln(q_v[0:RB, :].astype(F32))
    wait(4)
    kg = kgp(0)
    wprep(1); ln_rows(0, RB, q_v[0:RB, :].astype(F32), False, x_s[0:RB, :]); kg[0]()
    wait(5)
    kg[1](); t_hf(1, (0, 24)); t_kv(1, (0, -16)); t_h(1); t_u(1)
    wait(6)
    region(1, [F(wprep, 0)], Q(0), [(2, [1])], ln=(64,) * 4, lnt=90)
    for r in range(2, NR):
        if r in (2, 3, 5):
            wait({2: 7, 3: 8, 5: 9}[r])
        del ticks[:]; del loads[:]
        kg = kgp(r - 1)
        bw = [(r + 1, list(range(1, r + 1)))] if r + 1 < NR else []
        if r + 1 < NR:
            region(r, Q(r - 1), kg, bw, tail=TAIL if r in (2, 4) else 1)
        else:
            region(r, Q(r - 1, 0), kg + Q(r - 1, 1), nxt=False, ln=(64,) * 4)
    run(kgp(7))
    finalize(q_fill(NR - 1))

    def rows(i, n=RB):
        return pl.ds(pl.multiple_of(i * RB, RB), n)

    def att(qref, xref, rs):
        pq = _phi(qref[rs, :].astype(F32))
        t = pq * zr_s[0:1, :]
        t = (t[:, 0:128] + t[:, 128:256]) + (t[:, 256:384] + t[:, 384:512])
        t = t + pltpu.roll(t, 64, 1)
        t = t + pltpu.roll(t, 32, 1)
        den = t + 1e-6
        r = pl.reciprocal(den, approx=True)
        r = r * (2.0 - den * r)
        a = (pq * jnp.concatenate([r] * LT, axis=1)).astype(BF16)
        return xref[rs, :] + _dot(a, _upk(m_s[...]))

    def gate_ln(i, x, xout):
        cols = []
        for c in range(LT):
            b0 = c * S + i * RB
            lo = ldrev(lambda gg: ya[pl.ds(pl.multiple_of(b0 + gg * 8, 8), 8), :], HB)
            cols.append(jnp.concatenate([lo, ya[pl.ds(pl.multiple_of(b0 + HB, 8), HB), :]], axis=0))
        x = x + _ln(x) * jnp.concatenate(cols, axis=1)
        x2_s[rows(i), :] = x
        xout[...] = _pk(_ln(x).astype(BF16))

    def step(i):
        xa_s[...] = xb_s[...]
        pkt = _phi(_dot_nt(_upk(wqk_s[D // 2:D, :]), _upk(xb_s[...])))
        z_s[0:D, :] += pkt
        x = att(pq_s, x_s, rows(i + 1))
        q2_s[rows(i), :] = _dot_nt(_upk(xa_s[...]), _upk(wqk_s[0:D // 2, :])).astype(BF16)
        g_s[...] += _dot(pkt.astype(BF16), _upk(xa_s[...]))
        gate_ln(i + 1, x, xb_s)

    x0 = att(pq_s, x_s, rows(0))
    x1 = att(pq_s, x_s, rows(1))
    gate_ln(0, x0, xa_s)
    xc0 = lambda: _upk(xa_s[...])
    pkt = _phi(_dot_nt(_upk(wqk_s[D // 2:D, :]), xc0()))
    z_s[0:D, :] = pkt
    q2_s[rows(0), :] = _dot_nt(xc0(), _upk(wqk_s[0:D // 2, :])).astype(BF16)
    g_s[...] = _dot(pkt.astype(BF16), xc0())
    gate_ln(1, x1, xb_s)

    def body(it, carry):
        step(it)
        return carry
    lax.fori_loop(1, NR - 1, body, 0)
    xl = lambda: _upk(xb_s[...])
    pkt = _phi(_dot_nt(_upk(wqk_s[D // 2:D, :]), xl()))
    z_s[0:D, :] += pkt
    g_s[...] += _dot(pkt.astype(BF16), xl())

    def q_last(n0, n1):
        q2_s[S - RB:S, n0:n1] = _dot_nt(xl(), _upk(wqk_s[n0 // 2:n1 // 2, :])).astype(BF16)
    finalize([F(q_last, 0, 256), F(q_last, 256, 384), F(q_last, 384, 512)])

    chunks = [(i * RB, RB) for i in range(NR - 1)] + [(S - RB, 128), (S - 128, 128)]
    cps = []
    for r0, n in chunks:
        o_v[r0:r0 + n, :] = att(q2_s, x2_s, pl.ds(r0, n)).astype(BF16)
        cps.append(pltpu.make_async_copy(o_v.at[pl.ds(r0, n), :], o_hbm.at[0, pl.ds(r0, n), :], sem_o.at[0]))
        cps[-1].start()
    for cp in cps:
        cp.wait()


@jax.jit
def pallas_interleave_layers__ssm_conv_h3__linear_attn_block__prompt_kernel(
        A_q, A_k, A_v, A_shift_k, A_ssm_k, A_ssm_D, B_x, B_wqkv, B_wo):
    z = jnp.asarray(np.zeros((8,), np.int32))
    any_spec = pl.BlockSpec(memory_space=pl.ANY)
    return pl.pallas_call(
        _kernel,
        out_shape=jax.ShapeDtypeStruct((1, S, D), BF16),
        in_specs=[any_spec] * 9,
        out_specs=any_spec,
        scratch_shapes=[
            pltpu.VMEM((S, D), BF16),
            pltpu.VMEM((S, D), BF16),
            pltpu.VMEM((S, D), BF16),
            pltpu.VMEM((D, S), BF16),
            pltpu.VMEM((D, 3 * D), BF16),
            pltpu.VMEM((D, D), BF16),
            pltpu.VMEM((S, D), BF16),
            pltpu.VMEM((4, D), BF16),
            pltpu.VMEM((D,), BF16),
            pltpu.SMEM((8,), jnp.int32),
            pltpu.VMEM((C_ROWS // 2, 128), U32),
            pltpu.VMEM((LT, 8 + S, 128), F32),
            pltpu.VMEM((LT * HB, 128), F32),
            pltpu.VMEM((D + 8, RB), U32),
            pltpu.VMEM((NTICK * 8, 128), F32),
            pltpu.VMEM((PW_ROWS, 128), F32),
            pltpu.VMEM((ZB_ROWS, 256), U32),
            pltpu.VMEM((YA_ROWS, 128), F32),
            pltpu.VMEM((KVB_ROWS, 256), U32),
            pltpu.VMEM((4 * LT * 8 + 8, 128), F32),
            pltpu.VMEM((S // 2, D), U32),
            pltpu.VMEM((S, D), F32),
            pltpu.VMEM((S, D), BF16),
            pltpu.VMEM((D + 16, RB), BF16),
            pltpu.VMEM((D, D), F32),
            pltpu.VMEM((D + 8, RB), F32),
            pltpu.VMEM((D, D), U32),
            pltpu.VMEM((D // 2, D), U32),
            pltpu.VMEM((8, D), F32),
            pltpu.VMEM((RB // 2, D), U32),
            pltpu.VMEM((RB // 2, D), U32),
            pltpu.VMEM((S, D), F32),
            pltpu.VMEM((S, D), BF16),
            pltpu.SemaphoreType.DMA((10,)),
            pltpu.SemaphoreType.DMA((1,)),
        ] + [pltpu.VMEM((SP_ROWS, 128), F32)] * (2 * NR),
        compiler_params=pltpu.CompilerParams(vmem_limit_bytes=110 * 1024 * 1024),
    )(A_q, A_k, A_v, A_shift_k.T, A_ssm_k, A_ssm_D, B_wqkv, B_wo, z)
```

```python
import functools
import numpy as np
import jax
import jax.numpy as jnp
from jax import lax
import jax.experimental.pallas as pl
import jax.experimental.pallas.tpu as pltpu

S, D = 2048, 512
RB = 256
NR = S // RB
NFQ = 256
HB = RB // 2
DH = 16
LT = D // 128
HW = D // 2
F32 = jnp.float32
BF16 = jnp.bfloat16
U32 = jnp.uint32
TAIL = 14
LN_OPS = 1900.0


C_FH, C_OH, C_FU, C_CE, C_SO, C_PM, C_ROWS = 0, 512, 528, 1040, 1296, 1552, 1680


def _iota(shape, d):
    return lax.broadcasted_iota(jnp.int32, shape, d)


def _cossin(row_a, row_step, col, scale=None):
    nt, w = row_a.shape[0], col.shape[1]
    ang = lambda ph: (ph & 2047).astype(F32) * np.float32(np.pi / 1024.0)
    ta = ang(row_a * col)
    tb = ang(_iota((8, w), 0) * row_step * col)
    ca, sa, cb, sb = jnp.cos(ta), jnp.sin(ta), jnp.cos(tb), jnp.sin(tb)
    if scale is not None:
        cb, sb = cb * scale, sb * scale
    cs = [ca[t:t + 1] * cb - sa[t:t + 1] * sb for t in range(nt)]
    sn = [sa[t:t + 1] * cb + ca[t:t + 1] * sb for t in range(nt)]
    return jnp.concatenate(cs, axis=0), jnp.concatenate(sn, axis=0)


def _gen_consts(put):
    t = _iota((32, 1), 0)
    fa = 64 * (t % 8) + 2 * (t // 8) + 1
    p = _iota((1, 128), 1)
    c, sn = _cossin(fa, 8, jnp.where(p == 0, 2 * HB, 2 * p), jnp.full((1, 128), 2.0, F32))
    put(C_FH, c); put(C_FH + NFQ, -sn)
    put(C_OH, jnp.where(_iota((16, 128), 1) == 0, 2.0, 0.0))
    c, sn = _cossin(fa, 8, 2 * p + 1)
    put(C_FU, c); put(C_FU + NFQ, -sn)
    k = _iota((1, NFQ), 1)
    q = k // 64
    kf = jnp.where((q == 0) | (q == 3), 1.0, -1.0) * np.float32(np.sqrt(2.0) / (2 * RB))
    c, sn = _cossin(16 * _iota((16, 1), 0) + 1, 2, 8 * (k % 64) + 2 * q + 1, kf)
    put(C_CE, c[:, :128]); put(C_CE + 128, c[:, 128:]); put(C_SO, sn[:, :128]); put(C_SO + 128, sn[:, 128:])
    r, l = _iota((128, 128), 0), _iota((128, 128), 1)
    put(C_PM, jnp.where(l == (r % 8) * 16 + r // 8, 1.0, 0.0))


def _ln(x):
    m = jnp.mean(x, axis=-1, keepdims=True)
    xc = x - m
    v = jnp.mean(xc * xc, axis=-1, keepdims=True)
    return xc * jnp.exp(-0.5 * jnp.log(v + 1e-5))


def _phi(t):
    return jnp.where(t > 0, t + 1.0, jnp.exp(t)) + 1e-6


def _dot(a, b):
    return jnp.dot(a, b, preferred_element_type=F32)


def _dot_nt(a, b):
    return lax.dot_general(a, b, (((1,), (1,)), ((), ())), preferred_element_type=F32)


def _pk(x):
    return pltpu.bitcast(x, U32)


def _upk(x):
    return pltpu.bitcast(x, BF16)


AREA = 3 * NFQ + 8
SP_ROWS = LT * AREA
RAREA = 2 * NFQ + 8
NPART = 3
PW_ROWS = (1 + NPART) * LT * RAREA
YTOK = LT * S
YA_ROWS = YTOK + 8
KVB_ROWS = LT * (S // 4) + 8
ZB_ROWS = LT * (NFQ // 2) + 8
NTICK = 64 * 3 * NR


def _kernel(q_hbm, k_hbm, v_hbm, sk_hbm, h_hbm, sd_hbm, w_hbm, wo_hbm, z_hbm,
            o_hbm,
            q_v, k_v, v_v, h_v, w_v, wo_v, o_v, sk_v, sd_v, z_sm,
            cu_s, kf_s, kl_s, hf_s, tk_s, pw, zb, ya, kvb, skb, xn_s, x_s, pq_s, pk_s, g_s, z_s,
            wqk_s, m_s, zr_s, xa_s, xb_s, x2_s, q2_s,
            sem_in, sem_o, *spb):
    su, sh = spb[:NR], spb[NR:]

    def cp_rows(src, dst, i):
        return lambda s: pltpu.make_async_copy(src.at[0, pl.ds(i * RB, RB), :], dst.at[pl.ds(i * RB, RB), :], s)

    ck = lambda i: cp_rows(k_hbm, k_v, i)
    cv = lambda i: cp_rows(v_hbm, v_v, i)
    cq = lambda i: cp_rows(q_hbm, q_v, i)
    ch = lambda i, n=1: (lambda s: pltpu.make_async_copy(h_hbm.at[:, pl.ds(i * RB, n * RB)], h_v.at[:, pl.ds(i * RB, n * RB)], s))
    cw = lambda i: (lambda s: pltpu.make_async_copy(w_hbm.at[:, pl.ds(i * D, D)], w_v.at[:, pl.ds(i * D, D)], s))
    full = lambda a, b: (lambda s: pltpu.make_async_copy(a, b, s))
    groups = [
        [full(z_hbm, z_sm)],
        [ch(0), full(sd_hbm, sd_v)],
        [full(sk_hbm, sk_v), ck(0), cv(0)],
        [cq(0)],
        [cw(1)],
        [ch(1), ck(1), cv(1)],
        [cq(1), cw(0), ch(2), ck(2), cv(2)],
        [ch(3), ck(3), cv(3), cq(2)],
        [ch(4, 2), ck(4), cv(4), cq(3), ck(5), cv(5), cq(4)],
        [ch(6, 2), ck(6), cv(6), cq(5), ck(7), cv(7), cq(6), cq(7), cw(2), full(wo_hbm, wo_v)],
    ]
    for gi, g in enumerate(groups):
        for c in g:
            c(sem_in.at[gi]).start()

    ticks = []
    loads = []

    def wait(gi):
        for c in groups[gi]:
            c(sem_in.at[gi]).wait()
        del ticks[:]
        del loads[:]

    for c in range(LT):
        kf_s[c, 0:8, :] = jnp.zeros((8, 128), F32)

    def put_const(r, val):
        cu_s[r // 2:(r + val.shape[0]) // 2, :] = _pk(val.astype(BF16))

    _gen_consts(put_const)

    wait(0); wait(1)
    zero = z_sm[0]
    never = jnp.full((8, 128), zero, jnp.int32) != 0

    cm = lambda a, n: _upk(cu_s[a // 2:(a + n) // 2, :])
    cm2 = lambda a: jnp.concatenate([cm(a, 128), cm(a + 128, 128)], axis=1)

    def ldd(buf, r, n=8):
        return buf[pl.ds(pl.multiple_of(r + zero, 8), n), :]

    for b in spb:
        b[pl.ds(pl.multiple_of(3 * NFQ + zero, 8), 8), :] = jnp.zeros((8, 128), F32)
    pw[pl.ds(pl.multiple_of(2 * NFQ + zero, 8), 8), :] = jnp.zeros((8, 128), F32)
    kvb[pl.ds(pl.multiple_of(KVB_ROWS - 8 + zero, 8), 8), :] = jnp.zeros((8, 256), U32)
    zb[pl.ds(pl.multiple_of(ZB_ROWS - 8 + zero, 8), 8), :] = jnp.zeros((8, 256), U32)
    skb[pl.ds(pl.multiple_of(4 * LT * 8 + zero, 8), 8), :] = jnp.zeros((8, 128), F32)
    hf_s[pl.ds(pl.multiple_of(D + zero, 8), 8), :] = jnp.zeros((8, RB), U32)
    pk_s[pl.ds(pl.multiple_of(D + zero, 16), 16), :] = jnp.zeros((16, RB), BF16)
    z_s[pl.ds(pl.multiple_of(D + zero, 8), 8), :] = jnp.zeros((8, RB), F32)

    rev8 = 7 - lax.broadcasted_iota(jnp.int32, (8, 128), 0)

    def ldrev(load8, n):
        return jnp.concatenate([jnp.take_along_axis(load8(n // 8 - 1 - g), rev8, axis=0) for g in range(n // 8)], axis=0)

    def tick(val, order, load):
        for (r, c) in order:
            ticks.append(val[r * 8:(r + 1) * 8, c * 128:(c + 1) * 128])
            loads.append(float(load))

    def spread(n, cost, lo=0, hi=None):
        hi = len(ticks) if hi is None else (hi if hi >= 0 else len(ticks) + hi)
        need = n * cost
        a_, b_ = 0.0, 1e4
        for _ in range(60):
            lv = 0.5 * (a_ + b_)
            if sum(max(0.0, lv - loads[t]) for t in range(lo, hi)) < need:
                a_ = lv
            else:
                b_ = lv
        out, acc = [], 0.0
        for t in range(lo, hi):
            free = max(0.0, b_ - loads[t])
            while len(out) < n and acc + free > len(out) * cost:
                out.append(ticks[t])
            acc += free
            loads[t] = max(loads[t], b_)
        while len(out) < n:
            out.append(ticks[hi - 1])
        return out

    def sk_setup():
        skf = sk_v[...].astype(F32)
        for t in range(4):
            for c in range(LT):
                r = (t * LT + c) * 8
                skb[r:r + 8, :] = jnp.broadcast_to(skf[t:t + 1, c * 128:(c + 1) * 128], (8, 128))

    def kvrow(c, i):
        return (c * NR + i) * (HB // 2)

    def t_kv(i, win=None):
        r0 = i * RB
        kf = k_v[r0:r0 + RB, :].astype(F32)
        for c in range(LT):
            kf_s[c, 8 + r0:8 + r0 + RB, :] = kf[:, c * 128:(c + 1) * 128]
        items = [(hf, g) for hf in range(2) for g in range(HB // 32)]
        rel = spread(2 * len(items), 90.0, *win) if win is not None else None
        for k, (hf, g) in enumerate(items):
            bu, bl = r0 + HB + 32 * g, r0 + HB - 32 * (g + 1)
            vu = v_v[bu:bu + 32, hf * HW:(hf + 1) * HW].astype(F32)
            vl = v_v[bl:bl + 32, hf * HW:(hf + 1) * HW].astype(F32)
            for cl in range(2):
                c = 2 * hf + cl
                sk = [skb[(t * LT + c) * 8:(t * LT + c) * 8 + 8, :] for t in range(4)]
                if rel is not None:
                    sk = [jnp.where(never, rel[2 * k + cl], x) for x in sk]
                sk = [jnp.tile(x, (4, 1)) for x in sk]

                def kvof(b0, vf):
                    ks = (kf_s[c, 8 + b0:40 + b0, :] * sk[0] + kf_s[c, 7 + b0:39 + b0, :] * sk[1]
                          + kf_s[c, 6 + b0:38 + b0, :] * sk[2] + kf_s[c, 5 + b0:37 + b0, :] * sk[3])
                    return ks * vf[:, cl * 128:(cl + 1) * 128]
                up = kvof(bu, vu)
                lb = (c * (HB // 32) + g) * 32
                kl_s[lb:lb + 32, :] = kvof(bl, vl)
                lo = ldrev(lambda gg: kl_s[lb + gg * 8:lb + gg * 8 + 8, :], 32)
                r = kvrow(c, i) + g * 16
                kvb[r:r + 16, :] = _pk(jnp.concatenate([up + lo, up - lo], axis=1).astype(BF16))

    def put3(buf, hf, comps):
        val = jnp.stack(comps, axis=1).reshape(3 * NFQ, HW)
        for cl in range(2):
            r = (2 * hf + cl) * AREA
            buf[r:r + 3 * NFQ, :] = val[:, cl * 128:(cl + 1) * 128]

    def t_u(i):
        for hf in range(2):
            xe, xo = [jnp.concatenate([_upk(kvb[kvrow(c, i):kvrow(c, i) + HB // 2, eo * 128:(eo + 1) * 128])
                                       for c in (2 * hf, 2 * hf + 1)], axis=1) for eo in range(2)]
            ur = _dot(cm(C_FU, NFQ), xe)
            ui = _dot(cm(C_FU + NFQ, NFQ), xo)
            tick(ui, [(r, 0) for r in range(0, 32, 2)], 15)
            ur, ui = ur.reshape(16, 16, HW), ui.reshape(16, 16, HW)
            put3(su[i], hf, (ur, ui, ur + ui))

    lane = lax.broadcasted_iota(jnp.int32, (32, 128), 1)
    mirror = (128 - lane) % 128

    def t_hf(j, win=None):
        n = 32
        rel = spread(D // n, 30.0, *win) if win is not None else None
        for k in range(D // n):
            g = h_v[k * n:(k + 1) * n, j * RB:(j + 1) * RB].astype(F32)
            lo = jnp.take_along_axis(g[:, 0:128], mirror, axis=1)
            zz = jnp.zeros((8, 128), F32)
            if rel is not None:
                zz = jnp.where(never, rel[k], zz)
            up = jnp.where(lane == 0, jnp.tile(zz, (n // 8, 1)), g[:, 128:256])
            hf_s[((j % 2) * D + k * n) // 2:((j % 2) * D + (k + 1) * n) // 2, :] = _pk(
                jnp.concatenate([up + lo, up - lo], axis=1).astype(BF16))

    def t_h(j):
        for hf in range(2):
            r = ((j % 2) * D + hf * HW) // 2
            hb = _upk(hf_s[r:r + HW // 2, :])
            cen = _dot_nt(cm(C_OH, 16), h_v[hf * HW:(hf + 1) * HW, j * RB + 128:(j + 1) * RB])
            hr = _dot_nt(cm(C_FH, NFQ), hb[:, 0:128])
            hi = _dot_nt(cm(C_FH + NFQ, NFQ), hb[:, 128:256])
            tick(hi, [(r_, 0) for r_ in range(0, 32, 2)], 22)
            hr = hr.reshape(4, 4, 16, HW) + cen[None, None]
            hi = hi.reshape(4, 4, 16, HW)
            if j == 0:
                dd = sd_v[...].astype(F32).reshape(1, D)[:, hf * HW:(hf + 1) * HW] * np.float32(np.sqrt(2.0))
                hr = jnp.stack([hr[0] + dd, hr[1] - dd, hr[2] - dd, hr[3] + dd])
                hi = jnp.stack([hi[0] + dd, hi[1] + dd, hi[2] - dd, hi[3] - dd])
            hc = jnp.stack([hr[0] + hi[0], hr[1] - hi[1], hr[2] + hi[2], hr[3] - hi[3]]) * 0.5
            put3(sh[j], hf, tuple(x.reshape(16, 16, HW) for x in (hc, hr, hi)))

    def mac_slab(p, terms, first, last, c, q, t, link):
        base = c * AREA + t * 48
        lds = lambda buf, m: buf[pl.ds(pl.multiple_of(base + m * 16, 8), 16), :]
        even = q % 2 == 0
        rs = lambda slot, m: pl.ds(pl.multiple_of((slot * LT + c) * RAREA + t * 32 + m * 16, 8), 16)
        ps = 1 + p % NPART

        def chain(hm, um, acc, sign):
            for a in terms:
                tm = lds(sh[p - a], hm) * lds(su[a], um)
                acc = acc + tm if sign > 0 else acc - tm
            return acc

        if first:
            b0 = jnp.tile(jnp.where(never, link, jnp.zeros((8, 128), F32)), (2, 1))
        else:
            b0 = jnp.where(jnp.tile(never, (2, 1)), jnp.tile(link, (2, 1)), pw[rs(ps, 1), :])
        a0 = chain(1, 0, b0, -1) if even else chain(2, 0, b0, 1)
        wi = chain(0, 2, a0, 1)
        wr = chain(2 if even else 1, 1, wi - a0 if first else wi + (pw[rs(ps, 0), :] - a0), -1)
        if not last:
            pw[rs(ps, 0), :] = wr
            pw[rs(ps, 1), :] = wi
            return
        if p > 0:
            qr, qi = pw[rs(0, 0), :], pw[rs(0, 1), :]
            zr, zi = (wr - qi, wi + qr) if even else (wr + qi, wi - qr)
        else:
            zr, zi = wr, wi
        if p < NR - 1:
            pw[rs(0, 0), :] = wr
            pw[rs(0, 1), :] = wi
        zb[pl.ds(pl.multiple_of(c * (NFQ // 2) + t * 8, 8), 8), :] = _pk(jnp.concatenate([zr, zi], axis=1).astype(BF16))

    done = [[] for _ in range(NR)]
    ntk = [0]

    def mac(p, terms=None, win=None):
        if terms is None:
            terms = [a for a in list(range(1, p)) + ([0, p] if p > 0 else [0]) if a not in done[p]]
        first = not done[p]
        done[p] += list(terms)
        last = len(done[p]) == p + 1
        base = ntk[0]
        if win is not None:
            ntk[0] += 64
            for k, val in enumerate(spread(64, 12.0 * len(terms) + 10, *win)):
                tk_s[(base + k) * 8:(base + k + 1) * 8, :] = val
        link = jnp.zeros((8, 128), F32)
        for c in range(LT):
            for q in range(4):
                def body(tt, carry):
                    if win is not None:
                        carry = tk_s[pl.ds(pl.multiple_of((base + c * 16 + q * 4 + tt) * 8, 8), 8), :]
                    mac_slab(p, terms, first, last, c, q, q * 4 + tt, carry)
                    return carry
                lax.fori_loop(0, 4, body, link, unroll=True)

    def t_inv(i):
        for c in range(LT):
            zz = _upk(zb[c * (NFQ // 2):(c + 1) * (NFQ // 2), :])
            e = _dot(cm2(C_CE), zz[:, 0:128])
            o = _dot(cm2(C_SO), zz[:, 128:256])
            tick(o, [(r, 0) for r in range(0, 16, 2)], 8)
            r = c * S + i * RB
            ya[r:r + HB, :] = e + o
            ya[r + HB:r + RB, :] = e - o

    def get_y(r0, n, chained):
        ld = (lambda r, k: ldd(ya, r, k)) if chained else (lambda r, k: ya[r:r + k, :])
        blk, off = r0 // RB, r0 % RB
        cols = []
        for c in range(LT):
            b = c * S + blk * RB
            parts = []
            nl = max(0, min(off + n, HB) - off)
            if nl:
                s0 = b + HB - off - nl
                parts.append(ldrev(lambda gg: ld(s0 + gg * 8, 8), nl))
            if n - nl:
                parts.append(ld(b + off + nl, n - nl))
            cols.append(parts[0] if len(parts) == 1 else jnp.concatenate(parts, axis=0))
        return jnp.concatenate(cols, axis=1)

    def ln_rows(r0, n, x, chained, ln1=None):
        x = x + (_ln(x) if ln1 is None else ln1) * get_y(r0, n, chained)
        x_s[r0:r0 + n, :] = x
        xnf = _ln(x)
        xn_s[r0 // 2:(r0 + n) // 2, :] = _pk(xnf.astype(BF16))
        if chained:
            tok = xnf[0:8, 0:128]
            for g in range(1, n // 8):
                tok = tok + xnf[g * 8:(g + 1) * 8, (g % LT) * 128:(g % LT + 1) * 128]
            ya[YTOK:YTOK + 8, :] = tok

    def t_ln(i, sizes=(64,) * 4):
        r0 = i * RB
        for n in sizes:
            ln_rows(r0, n, q_v[r0:r0 + n, :].astype(F32), True)
            r0 += n

    def xn(i):
        return _upk(xn_s[i * RB // 2:(i + 1) * RB // 2, :])

    def q_half(i, h):
        r0 = i * RB
        qs = []
        for n in (2 * h, 2 * h + 1):
            qq = _dot_nt(xn(i), _upk(wqk_s[n * 64:(n + 1) * 64, :]))
            tick(qq, [(r, 0) for r in range(0, 32, 2)], 7)
            qs.append(qq)
        pq_s[r0:r0 + RB, h * HW:(h + 1) * HW] = jnp.concatenate(qs, axis=1).astype(BF16)

    def kgp(i):
        def kt():
            kt = _dot_nt(_upk(wqk_s[D // 2:D, :]), xn(i))
            tick(kt, [(r, c) for c in range(2) for r in range(0, D // 8, 2)], 19)
            pkt = _phi(kt)
            z_s[0:D, :] = pkt if i == 0 else z_s[0:D, :] + pkt
            for c in range(2):
                pk_s[0:D, c * 128:(c + 1) * 128] = pkt[:, c * 128:(c + 1) * 128].astype(BF16)

        def gm():
            gg = _dot(pk_s[0:D, :], xn(i))
            tick(gg, [(r, c) for c in (1, 3) for r in range(0, D // 8, 2)], 8)
            g_s[...] = gg if i == 0 else g_s[...] + gg
        return [kt, gm]

    def wprep(part):
        for gp in range(2):
            for hf in range(2):
                blk = [_dot_nt(cm(C_PM, 128), w_v[hf * HW:(hf + 1) * HW, part * D + g * 128: part * D + (g + 1) * 128])
                       for g in (2 * gp, 2 * gp + 1)]
                tick(blk[1], [(r, 0) for r in range(0, 16, 2)], 8)
                rows = jnp.stack([x.reshape(16, 8, HW) for x in blk], axis=1).reshape(256, HW)
                for e in range(16):
                    r = part * (D // 2) + e * 16 + gp * 8
                    wqk_s[r:r + 8, hf * HW:(hf + 1) * HW] = _pk(rows[e * 16:(e + 1) * 16].astype(BF16))

    def finalize(fill):
        zt = (z_s[0:D, 0:128] + z_s[0:D, 128:256]).T
        zr_s[...] = jnp.broadcast_to(jnp.sum(zt, axis=0, keepdims=True), (8, D))
        rr = lax.broadcasted_iota(jnp.int32, (128, 128), 0) % 8
        cc_ = lax.broadcasted_iota(jnp.int32, (128, 128), 1) // DH
        mask = rr == cc_
        fill[0]()
        kvs = []
        for g in range(4):
            gg = jnp.concatenate([g_s[e * 32 + g * 8: e * 32 + g * 8 + 8, :] for e in range(16)], axis=0).astype(BF16)
            wv = w_v[:, 2 * D + g * 128: 2 * D + (g + 1) * 128]
            kvs.append(jnp.where(mask, _dot(gg, wv), 0.0).astype(BF16))
        fill[1]()
        ms = [_dot(kvs[g], wo_v[g * 128:(g + 1) * 128, :]) for g in range(4)]
        for e in range(16):
            rows = jnp.concatenate([ms[g][e * 8:(e + 1) * 8] for g in range(4)], axis=0)
            m_s[e * 16:(e + 1) * 16, :] = _pk(rows.astype(BF16))
        fill[2]()

    def q_cols(i, n0, n1):
        r0 = i * RB
        pq_s[r0:r0 + RB, n0:n1] = _dot_nt(xn(i), _upk(wqk_s[n0 // 2:n1 // 2, :])).astype(BF16)

    def q_fill(i):
        return [functools.partial(q_cols, i, 0, 256), functools.partial(q_cols, i, 256, 384), functools.partial(q_cols, i, 384, 512)]

    F = functools.partial
    Q = lambda i, *hs: [F(q_half, i, h) for h in (hs or (0, 1))]

    def run(ts):
        for t in ts:
            t()

    def region(r, pre, post, bwork=(), nxt=True, ln=(32,) * 8, lnt=170, tail=TAIL):
        run(pre)
        mac(r, None, (0, -4))
        t_inv(r)
        t1 = len(ticks)
        run(post)
        for t in range(t1 - 8, min(len(ticks), t1 - 8 + lnt)):
            loads[t] += LN_OPS / lnt
        if nxt:
            t_kv(r + 1, (0, -10))
            t_hf(r + 1, (0, -10))
            t_h(r + 1); t_u(r + 1)
        for p_, terms in bwork:
            mac(p_, terms, (0, -tail))
        t_ln(r, ln)

    t_hf(0); t_h(0)
    wait(2)
    sk_setup(); t_kv(0)
    wait(3)
    t_u(0); mac(0); t_inv(0)
    x_s[0:RB, :] = _ln(q_v[0:RB, :].astype(F32))
    wait(4)
    kg = kgp(0)
    wprep(1); ln_rows(0, RB, q_v[0:RB, :].astype(F32), False, x_s[0:RB, :]); kg[0]()
    wait(5)
    kg[1](); t_hf(1, (0, 24)); t_kv(1, (0, -16)); t_h(1); t_u(1)
    wait(6)
    region(1, [F(wprep, 0)], Q(0), [(2, [1])], ln=(64,) * 4, lnt=90)
    for r in range(2, NR):
        if r in (2, 3, 5):
            wait({2: 7, 3: 8, 5: 9}[r])
        del ticks[:]; del loads[:]
        kg = kgp(r - 1)
        bw = [(r + 1, list(range(1, r + 1)))] if r + 1 < NR else []
        if r + 1 < NR:
            region(r, Q(r - 1), kg, bw, tail=TAIL if r in (2, 4) else 1)
        else:
            region(r, kg[:1], kg[1:] + Q(r - 1, 0), nxt=False, ln=(64,) * 4)
    run(kgp(7))
    finalize(q_fill(NR - 1))
    g_s[...] = jnp.zeros_like(g_s)
    z_s[0:D, :] = jnp.zeros((D, RB), F32)

    def rows(i, n=RB):
        return pl.ds(pl.multiple_of(i * RB, RB), n)

    def att(qref, xref, rs):
        pq = _phi(qref[rs, :].astype(F32))
        t = pq * zr_s[0:1, :]
        t = (t[:, 0:128] + t[:, 128:256]) + (t[:, 256:384] + t[:, 384:512])
        t = t + pltpu.roll(t, 64, 1)
        t = t + pltpu.roll(t, 32, 1)
        den = t + 1e-6
        r = pl.reciprocal(den, approx=True)
        r = r * (2.0 - den * r)
        a = (pq * jnp.concatenate([r] * LT, axis=1)).astype(BF16)
        return xref[rs, :] + _dot(a, _upk(m_s[...]))

    def gate_ln(i, x, xout):
        cols = []
        for c in range(LT):
            b0 = c * S + i * RB
            lo = ldrev(lambda gg: ya[pl.ds(pl.multiple_of(b0 + gg * 8, 8), 8), :], HB)
            cols.append(jnp.concatenate([lo, ya[pl.ds(pl.multiple_of(b0 + HB, 8), HB), :]], axis=0))
        x = x + _ln(x) * jnp.concatenate(cols, axis=1)
        x2_s[rows(i), :] = x
        xout[...] = _pk(_ln(x).astype(BF16))

    def step(i):
        xa_s[...] = xb_s[...]
        pkt = _phi(_dot_nt(_upk(wqk_s[D // 2:D, :]), _upk(xb_s[...])))
        z_s[0:D, :] += pkt
        x = att(pq_s, x_s, rows(i + 1))
        q2_s[rows(i), :] = _dot_nt(_upk(xa_s[...]), _upk(wqk_s[0:D // 2, :])).astype(BF16)
        g_s[...] += _dot(pkt.astype(BF16), _upk(xa_s[...]))
        gate_ln(i + 1, x, xb_s)

    x0 = att(pq_s, x_s, rows(0))
    q_cols(NR - 2, HW, D)
    gate_ln(0, x0, xb_s)

    def body(it, carry):
        step(it)
        return carry
    lax.fori_loop(0, NR - 1, body, 0)
    xl = lambda: _upk(xb_s[...])
    pkt = _phi(_dot_nt(_upk(wqk_s[D // 2:D, :]), xl()))
    z_s[0:D, :] += pkt
    g_s[...] += _dot(pkt.astype(BF16), xl())

    def q_last(n0, n1):
        q2_s[S - RB:S, n0:n1] = _dot_nt(xl(), _upk(wqk_s[n0 // 2:n1 // 2, :])).astype(BF16)
    finalize([F(q_last, 0, 256), F(q_last, 256, 384), F(q_last, 384, 512)])

    chunks = [(i * RB, RB) for i in range(NR - 1)] + [(S - RB, 128), (S - 128, 128)]
    cps = []
    for r0, n in chunks:
        o_v[r0:r0 + n, :] = att(q2_s, x2_s, pl.ds(r0, n)).astype(BF16)
        cps.append(pltpu.make_async_copy(o_v.at[pl.ds(r0, n), :], o_hbm.at[0, pl.ds(r0, n), :], sem_o.at[0]))
        cps[-1].start()
    for cp in cps:
        cp.wait()


@jax.jit
def pallas_interleave_layers__ssm_conv_h3__linear_attn_block__prompt_kernel(
        A_q, A_k, A_v, A_shift_k, A_ssm_k, A_ssm_D, B_x, B_wqkv, B_wo):
    z = jnp.asarray(np.zeros((8,), np.int32))
    any_spec = pl.BlockSpec(memory_space=pl.ANY)
    return pl.pallas_call(
        _kernel,
        out_shape=jax.ShapeDtypeStruct((1, S, D), BF16),
        in_specs=[any_spec] * 9,
        out_specs=any_spec,
        scratch_shapes=[
            pltpu.VMEM((S, D), BF16),
            pltpu.VMEM((S, D), BF16),
            pltpu.VMEM((S, D), BF16),
            pltpu.VMEM((D, S), BF16),
            pltpu.VMEM((D, 3 * D), BF16),
            pltpu.VMEM((D, D), BF16),
            pltpu.VMEM((S, D), BF16),
            pltpu.VMEM((4, D), BF16),
            pltpu.VMEM((D,), BF16),
            pltpu.SMEM((8,), jnp.int32),
            pltpu.VMEM((C_ROWS // 2, 128), U32),
            pltpu.VMEM((LT, 8 + S, 128), F32),
            pltpu.VMEM((LT * HB, 128), F32),
            pltpu.VMEM((D + 8, RB), U32),
            pltpu.VMEM((NTICK * 8, 128), F32),
            pltpu.VMEM((PW_ROWS, 128), F32),
            pltpu.VMEM((ZB_ROWS, 256), U32),
            pltpu.VMEM((YA_ROWS, 128), F32),
            pltpu.VMEM((KVB_ROWS, 256), U32),
            pltpu.VMEM((4 * LT * 8 + 8, 128), F32),
            pltpu.VMEM((S // 2, D), U32),
            pltpu.VMEM((S, D), F32),
            pltpu.VMEM((S, D), BF16),
            pltpu.VMEM((D + 16, RB), BF16),
            pltpu.VMEM((D, D), F32),
            pltpu.VMEM((D + 8, RB), F32),
            pltpu.VMEM((D, D), U32),
            pltpu.VMEM((D // 2, D), U32),
            pltpu.VMEM((8, D), F32),
            pltpu.VMEM((RB // 2, D), U32),
            pltpu.VMEM((RB // 2, D), U32),
            pltpu.VMEM((S, D), F32),
            pltpu.VMEM((S, D), BF16),
            pltpu.SemaphoreType.DMA((10,)),
            pltpu.SemaphoreType.DMA((1,)),
        ] + [pltpu.VMEM((SP_ROWS, 128), F32)] * (2 * NR),
        compiler_params=pltpu.CompilerParams(vmem_limit_bytes=110 * 1024 * 1024),
    )(A_q, A_k, A_v, A_shift_k.T, A_ssm_k, A_ssm_D, B_wqkv, B_wo, z)
```
